```python
import os as _os
_os.environ.setdefault("JAX_PLATFORMS", "cpu")
import jax
import jax.numpy as jnp

def _softmax(x, axis=-1):
    return jax.nn.softmax(x, axis=axis)
def _gelu(x):
    return jax.nn.gelu(x, approximate=True)
def _silu(x):
    return jax.nn.silu(x)
def _sigmoid(x):
    return jax.nn.sigmoid(x)
def _layernorm(x, axis=-1, eps=1e-5):
    m = jnp.mean(x, axis=axis, keepdims=True)
    v = jnp.var(x, axis=axis, keepdims=True)
    return (x - m) / jnp.sqrt(v + eps)
def _scatter_add(tgt, idx, src, axis=0):
    return tgt.at[idx].add(src)
def _segment_sum(src, seg, n):
    return jax.ops.segment_sum(src, seg, n)
class _Rng:
    def __init__(self, key):
        self._k = key
    def _next(self):
        self._k, sub = jax.random.split(self._k)
        return sub
    def normal(self, shape):
        return jax.random.normal(self._next(), shape, dtype=jnp.bfloat16)
    def randint(self, lo, hi, shape):
        return jax.random.randint(self._next(), shape, lo, hi, dtype=jnp.int32)
    def uniform(self, shape, lo=0.0, hi=1.0):
        return jax.random.uniform(self._next(), shape, jnp.bfloat16, lo, hi)
    def permutation(self, n):
        return jax.random.permutation(self._next(), n)


kernel_name = 'concat_heads__gqa_block_cached__mha_block_cached__near_ridge'

def setup_inputs():
    _rng = _Rng(jax.random.key(int.from_bytes(__import__("os").urandom(4), "little")))
    _w = (lambda a: (lambda t: t.astype(jnp.bfloat16) if jnp.issubdtype(t.dtype, jnp.floating) else t)(jnp.asarray(a)))
    def _A_setup():
        B, Sq, D = 8, 112, 448
        Hq, Hkv, Sk, Dh = 16, 8, 512, 256
        assert Hq % Hkv == 0, (Hq, Hkv)
        return {
            "x": _w((lambda *s: _rng.normal(s) * 0.8)(B, Sq, D)),
            "k_cache": _w((lambda *s: _rng.normal(s) * 0.8)(B, Hkv, Sk, Dh)),
            "v_cache": _w((lambda *s: _rng.normal(s) * 0.05)(B, Hkv, Sk, Dh)),
            "wq": _w((lambda *s: _rng.normal(s) * 0.8)(D, Hq * Dh) * (D ** -0.5)),
            "wo": _w((lambda *s: _rng.normal(s) * 0.05)(Hq * Dh, D) * ((Hq * Dh) ** -0.5)),
        }
    _A_in = _A_setup()

    def _B_setup():
        B, Sq, D = 8, 112, 448
        H, Sk, Dh = 16, 512, 256
        return {
            "x": _w((lambda *s: _rng.normal(s) * 0.8)(B, Sq, D)),
            "k_cache": _w((lambda *s: _rng.normal(s) * 0.8)(B, H, Sk, Dh)),
            "v_cache": _w((lambda *s: _rng.normal(s) * 0.05)(B, H, Sk, Dh)),
            "wq": _w((lambda *s: _rng.normal(s) * 0.8)(D, H * Dh) * (D ** -0.5)),
            "wo": _w((lambda *s: _rng.normal(s) * 0.05)(H * Dh, D) * ((H * Dh) ** -0.5)),
        }
    _B_in = _B_setup()

    return {
        "A_x": _A_in["x"],
        "A_k_cache": _A_in["k_cache"],
        "A_v_cache": _A_in["v_cache"],
        "A_wq": _A_in["wq"],
        "A_wo": _A_in["wo"],
        "B_x": _B_in["x"],
        "B_k_cache": _B_in["k_cache"],
        "B_v_cache": _B_in["v_cache"],
        "B_wq": _B_in["wq"],
        "B_wo": _B_in["wo"],
    }

def reference(A_x, A_k_cache, A_v_cache, A_wq, A_wo, B_x, B_k_cache, B_v_cache, B_wq, B_wo):
    def _A_ref(x, k_cache, v_cache, wq, wo):
        B, Sq, D = x.shape
        Hq, Dh = 16, 256
        Hkv = k_cache.shape[1]
        rep = Hq // Hkv
        q = (lambda x, *d: x.transpose(*d))((x @ wq).reshape(B, Sq, Hq, Dh), 0, 2, 1, 3)
        k = jnp.repeat(k_cache, rep, axis=1)
        v = jnp.repeat(v_cache, rep, axis=1)
        scores = jnp.einsum("bhqd,bhkd->bhqk", q, k) * (Dh ** -0.5)
        p = _softmax(scores, axis=-1)
        o = jnp.einsum("bhqk,bhkd->bhqd", p, v)
        return (lambda x, *d: x.transpose(*d))(o, 0, 2, 1, 3).reshape(B, Sq, Hq * Dh) @ wo

    def _B_ref(x, k_cache, v_cache, wq, wo):
        B, Sq, D = x.shape
        H, Dh = 16, 256
        q = (lambda x, *d: x.transpose(*d))((x @ wq).reshape(B, Sq, H, Dh), 0, 2, 1, 3)
        scores = jnp.einsum("bhqd,bhkd->bhqk", q, k_cache) * (Dh ** -0.5)
        p = _softmax(scores, axis=-1)
        o = jnp.einsum("bhqk,bhkd->bhqd", p, v_cache)
        return (lambda x, *d: x.transpose(*d))(o, 0, 2, 1, 3).reshape(B, Sq, H * Dh) @ wo

    a = _A_ref(A_x, A_k_cache, A_v_cache, A_wq, A_wo)
    b = _B_ref(B_x, B_k_cache, B_v_cache, B_wq, B_wo)
    return jnp.concatenate([a, b], axis=-1)
```

```python
import functools, contextlib
import jax
import jax.numpy as jnp
from jax import lax
import jax.experimental.pallas as pl
import jax.experimental.pallas.tpu as pltpu

LOG2E = 1.4426950408889634
NT = (((1,), (1,)), ((), ()))

def make(NS=16, LA=14, scr=True, scopes=False, order=0, tail=0):
    @jax.jit
    def kernel(A_x, A_k_cache, A_v_cache, A_wq, A_wo, B_x, B_k_cache, B_v_cache, B_wq, B_wo):
        B, Sq, D = A_x.shape
        Hq, Dh = 16, 256
        NJ, Sk = A_k_cache.shape[1], A_k_cache.shape[2]
        rep = Hq // NJ
        W = rep * Dh
        R = B * Sq
        NTL = R // 128
        U = 2
        qscale = (Dh ** -0.5) * LOG2E
        assert NS >= LA + U and LA == 2 * NJ - 2
        IPJ = B // U
        NSTEP = NJ * B
        NIT = NSTEP // U
        UK = 256
        LAG = 2
        PR = D // B
        H = R // 2
        bf16 = jnp.bfloat16
        S_X = 0
        S_WQ = 4
        S_WO = S_WQ + 2 * NJ
        S_K = S_WO + NJ
        S_V = S_K + NS
        S_OUT = S_V + NS
        NSEM = S_OUT + NTL

        def scope(name):
            return jax.named_scope(name) if scopes else contextlib.nullcontext()

        xa = A_x.reshape(R, D)
        xb = B_x.reshape(R, D)
        woa_t = A_wo.T
        wob_t = B_wo.T

        def body(xa_h, ka_h, va_h, wqa_h, woa_h, xb_h, kb_h, vb_h, wqb_h, wob_h, out_h,
                 x_v, wq_v, wo_v, ka_v, va_v, kb_v, vb_v, q_v, o_v, acc_v, ost_v, s_v, p_v, sem):
            x_h = (xa_h, xb_h); wq_h = (wqa_h, wqb_h); wo_h = (woa_h, wob_h)

            def split(s):
                if isinstance(s, int):
                    return s // B, s % B, s % NS
                return lax.shift_right_logical(s, 3), s & (B - 1), s & (NS - 1)

            def k_copies(s):
                j, b, slot = split(s)
                sm = sem.at[S_K + slot]
                return (pltpu.make_async_copy(ka_h.at[b, j], ka_v.at[slot], sm),
                        pltpu.make_async_copy(kb_h.at[b, pl.ds(j * rep, rep)], kb_v.at[slot], sm))

            def v_copies(s):
                j, b, slot = split(s)
                sm = sem.at[S_V + slot]
                return (pltpu.make_async_copy(va_h.at[b, j], va_v.at[slot], sm),
                        pltpu.make_async_copy(vb_h.at[b, pl.ds(j * rep, rep)], vb_v.at[slot], sm))

            def kv_start(s):
                for c in k_copies(s) + v_copies(s): c.start()

            def x_copy(br, half):
                rows = pl.ds(half * H, H)
                return pltpu.make_async_copy(x_h[br].at[rows], x_v.at[br, rows], sem.at[S_X + 2 * br + half])

            def wq_copy(br, j, src=None):
                cols = pl.ds(pl.multiple_of(j * W, W), W)
                return pltpu.make_async_copy(wq_h[br if src is None else src].at[:, cols], wq_v.at[br, j], sem.at[S_WQ + br * NJ + j])

            def wo_copy(br, j, p=None):
                cols = pl.ds(pl.multiple_of(j * W, W), W)
                sm = sem.at[S_WO + j]
                if p is None:
                    return pltpu.make_async_copy(wo_h[br].at[:, cols], wo_v.at[j, br], sm)
                rows = pl.ds(pl.multiple_of(p * PR, 8), PR)
                return pltpu.make_async_copy(wo_h[br].at[rows, cols], wo_v.at[j, br, rows], sm)

            def out_copy(t):
                return pltpu.make_async_copy(ost_v.at[t], out_h.at[pl.ds(t * 128, 128)], sem.at[S_OUT + t])

            def stream_start(s):
                kv_start(s)
                j, b, _ = split(s)
                if isinstance(s, int):
                    if j + 1 < NJ:
                        for br in range(2): wo_copy(br, j + 1, b).start()
                else:
                    @pl.when(j + 1 < NJ)
                    def _():
                        for br in range(2): wo_copy(br, j + 1, b).start()

            wq_copy(0, 0).start()
            x_copy(0, 0).start()
            x_copy(0, 1).start()
            for j in range(1, NJ): wq_copy(0, j).start()
            x_copy(1, 0).start()
            x_copy(1, 1).start()
            for j in range(NJ): wq_copy(1, j).start()
            for br in range(2): wo_copy(br, 0).start()

            acc_v[...] = jnp.zeros(acc_v.shape, acc_v.dtype)

            def qproj(br, j, b0, nb):
                r0 = b0 * Sq
                q = (jnp.dot(x_v[br, pl.ds(r0, nb * Sq), :], wq_v[br, j], preferred_element_type=jnp.float32) * qscale).astype(bf16)
                for bb in range(nb):
                    for h in range(rep):
                        q_v[br, j, b0 + bb, h] = q[bb * Sq:(bb + 1) * Sq, h * Dh:(h + 1) * Dh]

            with scope('S_p1a'):
                wq_copy(0, 0).wait()
                x_copy(0, 0).wait()
                qproj(0, 0, 0, B // 2)
                x_copy(0, 1).wait()
                qproj(0, 0, B // 2, B // 2)

            def p1(c, carry):
                br = lax.shift_right_logical(c, 3)
                j = c & (NJ - 1)
                @pl.when(c == NJ)
                def _():
                    x_copy(1, 0).wait()
                    x_copy(1, 1).wait()
                wq_copy(br, j, src=0).wait()
                kv_start(c - 1)
                jn, bn, _ = split(c - 1)
                for b2 in range(2): wo_copy(b2, jn + 1, bn).start()
                qproj(br, j, 0, B)
                return carry
            with scope('S_p1'):
                lax.fori_loop(1, 2 * NJ - 1, p1, 0)
            wq_copy(1, NJ - 1).wait()

            HD = D // 2
            def ounit(jj, t, br, rh, nr):
                if isinstance(t, int):
                    r0, w0 = t * 128, rh * HD
                    d0 = br * D + w0
                else:
                    r0 = pl.multiple_of(t * 128, 128)
                    w0 = pl.multiple_of(rh * HD, 16)
                    d0 = pl.multiple_of(br * D + w0, 8)
                ot = o_v[br, pl.ds(r0, 128), :]
                lhs = wo_v[jj, br, pl.ds(w0, nr), :]
                acc_v[t, pl.ds(d0, nr), :] += lax.dot_general(lhs, ot, NT, preferred_element_type=jnp.float32)

            def hunit(jj, u):
                t = lax.shift_right_logical(u, 2)
                br = lax.shift_right_logical(u, 1) & 1
                ounit(jj, t, br, u & 1, HD)

            def group(jj, t, br):
                ounit(jj, t, br, 0, D)

            def finalize(t):
                ost_v[t] = acc_v[t].T.astype(bf16)
                out_copy(t).start()

            def QK(s, k):
                j, b, slot = split(s)
                qs = [q_v[0, j, b].reshape(rep * Sq, Dh)] + [q_v[1, j, b, h] for h in range(rep)]
                ks = [ka_v[slot]] + [kb_v[slot, h] for h in range(rep)]
                res = []
                r0 = 0
                for q, kk in zip(qs, ks):
                    sc = lax.dot_general(q, kk, NT, preferred_element_type=jnp.float32)
                    m = jnp.max(sc, axis=-1, keepdims=True)
                    n = q.shape[0]
                    if scr:
                        s_v[k, r0:r0 + n, :] = sc
                        sc = None
                    res.append((sc, m, r0, n))
                    r0 += n
                return (s, k, res)

            def SM(st):
                s, k, res = st
                out = []
                for (sc, m, r0, n) in res:
                    if scr:
                        sc = s_v[k, r0:r0 + n, :]
                    p = jnp.exp2(sc - m)
                    l = jnp.sum(p, axis=-1, keepdims=True)
                    p = p.astype(bf16)
                    if scr:
                        for c in range(Sk // 128):
                            p_v[k, c, r0:r0 + n, :] = p[:, c * 128:(c + 1) * 128]
                        p = None
                    out.append((p, 1.0 / l, r0, n))
                return (s, k, out)

            def PV(st, which=(0, 1, 2)):
                s, k, res = st
                j, b, slot = split(s)
                rows = pl.ds(b * Sq if isinstance(b, int) else pl.multiple_of(b * Sq, 16), Sq)
                for idx in which:
                    p, r, r0, n = res[idx]
                    v = va_v[slot] if idx == 0 else vb_v[slot, idx - 1]
                    if scr:
                        p = jnp.concatenate([p_v[k, c, r0:r0 + n, :] for c in range(Sk // 128)], axis=1)
                    o = (jnp.dot(p, v, preferred_element_type=jnp.float32) * r).astype(bf16)
                    if idx == 0:
                        for h in range(rep):
                            o_v[0, rows, h * Dh:(h + 1) * Dh] = o[h * Sq:(h + 1) * Sq]
                    else:
                        o_v[1, rows, (idx - 1) * Dh:idx * Dh] = o

            def kv_wait(s):
                for c in k_copies(s) + v_copies(s): c.wait()

            def issue(n):
                s1 = n * U + LA
                @pl.when(s1 < NSTEP)
                def _():
                    for k in range(U): kv_start(s1 + k)
                @pl.when(s1 < NSTEP - B)
                def _():
                    for k in range(U):
                        j1, b1, _ = split(s1 + k)
                        for br in range(2): wo_copy(br, j1 + 1, b1).start()

            def p2a(n, carry):
                s = n * U
                kv_wait(s); kv_wait(s + 1)
                a = QK(s, 0)
                b_ = QK(s + 1, 1)
                qproj(1, NJ - 1, n * (B // 2), B // 2)
                PV(SM(a))
                issue(n)
                PV(SM(b_))
                return carry
            with scope('S_p2a'):
                if True:
                    for n in range(LAG):
                        p2a(n, 0)

            def p2b(n, carry):
                s = n * U
                nu = n - LAG
                jj = lax.shift_right_logical(nu, 2)
                u0 = (nu & (IPJ - 1)) * 7
                @pl.when(u0 == 0)
                def _():
                    for br in range(2): wo_copy(br, jj).wait()
                kv_wait(s); kv_wait(s + 1)
                if order == 0:
                    a = QK(s, 0)
                    for i in range(4): hunit(jj, u0 + i)
                    b_ = QK(s + 1, 1)
                    for i in range(4, 7): hunit(jj, u0 + i)
                    PV(SM(a))
                    issue(n)
                    PV(SM(b_))
                elif order == 1:
                    a = QK(s, 0)
                    b_ = QK(s + 1, 1)
                    for i in range(4): hunit(jj, u0 + i)
                    PV(SM(a))
                    issue(n)
                    PV(SM(b_))
                    for i in range(4, 7): hunit(jj, u0 + i)
                elif order == 2:
                    a = QK(s, 0)
                    for i in range(2): hunit(jj, u0 + i)
                    b_ = QK(s + 1, 1)
                    for i in range(2, 4): hunit(jj, u0 + i)
                    sa = SM(a)
                    PV(sa, (0,))
                    for i in range(4, 7): hunit(jj, u0 + i)
                    PV(sa, (1, 2))
                    issue(n)
                    PV(SM(b_))
                return carry
            with scope('S_p2b'):
                lax.fori_loop(LAG, NIT - 2, p2b, 0)

            jl = NJ - 1
            s0 = NSTEP - 4
            with scope('S_p3'):
                for br in range(2): wo_copy(br, jl).wait()
                gl = [(t, br) for t in range(NTL) for br in range(2)]
                for k in range(3):
                    s = s0 + k
                    kv_wait(s)
                    a = QK(s, 0)
                    for (t, br) in gl[3 * k:3 * k + 3]: group(jl, t, br)
                    if k >= 1: finalize(k - 1)
                    PV(SM(a))
                for (t, br) in gl[9:12]: group(jl, t, br)
                finalize(2); finalize(3)
                s = NSTEP - 1
                for c in k_copies(s): c.wait()
                a = SM(QK(s, 0))
                finalize(4); finalize(5)
                for c in v_copies(s): c.wait()
                PV(a)
                group(jl, 6, 0); group(jl, 6, 1)
                finalize(6)
                for t in range(NTL):
                    out_copy(t).wait()

        ms = pltpu.HBM
        out = pl.pallas_call(
            body,
            in_specs=[pl.BlockSpec(memory_space=ms)] * 10,
            out_specs=pl.BlockSpec(memory_space=ms),
            out_shape=jax.ShapeDtypeStruct((R, 2 * D), A_x.dtype),
            scratch_shapes=[
                pltpu.VMEM((2, R, D), bf16),
                pltpu.VMEM((2, NJ, D, W), bf16),
                pltpu.VMEM((NJ, 2, D, W), bf16),
                pltpu.VMEM((NS, Sk, Dh), bf16),
                pltpu.VMEM((NS, Sk, Dh), bf16),
                pltpu.VMEM((NS, rep, Sk, Dh), bf16),
                pltpu.VMEM((NS, rep, Sk, Dh), bf16),
                pltpu.VMEM((2, NJ, B, rep, Sq, Dh), bf16),
                pltpu.VMEM((2, R, W), bf16),
                pltpu.VMEM((NTL, 2 * D, 128), jnp.float32),
                pltpu.VMEM((NTL, 128, 2 * D), bf16),
                pltpu.VMEM((U, 2 * rep * Sq, Sk), jnp.float32),
                pltpu.VMEM((U, Sk // 128, 2 * rep * Sq, 128), bf16),
                pltpu.SemaphoreType.DMA((NSEM,)),
            ],
            compiler_params=pltpu.CompilerParams(vmem_limit_bytes=110 * 1024 * 1024,
                                                 disable_bounds_checks=True, disable_semaphore_checks=True),
        )(xa, A_k_cache, A_v_cache, A_wq, woa_t, xb, B_k_cache, B_v_cache, B_wq, wob_t)
        return out.reshape(B, Sq, 2 * D)
    return kernel


_impl = make(order=0)


@jax.jit
def pallas_concat_heads__gqa_block_cached__mha_block_cached__near_ridge_kernel(A_x, A_k_cache, A_v_cache, A_wq, A_wo, B_x, B_k_cache, B_v_cache, B_wq, B_wo):
    return _impl(A_x, A_k_cache, A_v_cache, A_wq, A_wo, B_x, B_k_cache, B_v_cache, B_wq, B_wo)
```

```python
import functools, contextlib
import jax
import jax.numpy as jnp
from jax import lax
import jax.experimental.pallas as pl
import jax.experimental.pallas.tpu as pltpu

LOG2E = 1.4426950408889634
NT = (((1,), (1,)), ((), ()))


def make(L=9, scopes=False, pa_units=4, p1c=2, late_out=True):
    @jax.jit
    def kernel(A_x, A_k_cache, A_v_cache, A_wq, A_wo, B_x, B_k_cache, B_v_cache, B_wq, B_wo):
        B, Sq, D = A_x.shape
        Hq, Dh = 16, 256
        NJ, Sk = A_k_cache.shape[1], A_k_cache.shape[2]
        rep = Hq // NJ
        W = rep * Dh
        R = B * Sq
        NTL = R // 128
        qscale = (Dh ** -0.5) * LOG2E
        PPJ = B // 2
        NP = NJ * PPJ
        DP = PPJ
        NSP = 16
        assert L + 1 <= NSP
        HD = D // 2
        PR = D // PPJ
        H = R // 2
        KC = Sk // 128
        bf16 = jnp.bfloat16
        S_X = 0
        S_WQ = 4
        S_WO = S_WQ + 2 * NJ
        S_A = S_WO + 2 * NJ
        S_B = S_A + NSP
        S_F = S_B + NSP
        S_OUT = S_F + 4
        NSEM = S_OUT + NTL
        UPB = 7

        def build(counts):
            queue, pushed, out = [], [0, 0], []
            for (n, da, db, ea, eb) in counts:
                for br, done in ((0, da), (1, db)):
                    ready = (done // B) * NTL + max(0, done % B - 1)
                    while pushed[br] < ready:
                        j, t = divmod(pushed[br], NTL)
                        pushed[br] += 1
                        queue += [(br, j, t, 0), (br, j, t, 1)]
                queue.sort(key=lambda u: (u[1] * B + u[2] - (DP * 2 if u[0] == 0 else 0), u[0], u[3]))
                if n < 0: n = len(queue)
                assert len(queue) >= n, (counts, len(out))
                out.append(queue[:n]); queue = queue[n:]
                for (br, j, t, rh) in queue:
                    assert (ea, eb)[br] <= (j + 1) * B + t, "o rows overwritten"
            assert not queue and pushed == [NJ * NTL] * 2
            return out
        NS_ = NJ * B
        counts = [(0, 0, 0, 4, 0), (pa_units, 4, 0, 8, 0)]
        for m in range(NP - DP):
            counts.append((UPB, 2 * (m + DP), 2 * m, 2 * (m + DP + 1), 2 * (m + 1)))
        for sB, eB in ((56, 58), (58, 60), (60, 62), (62, 63), (63, 63), (64, 64)):
            counts.append((-1, NS_, sB, NS_, eB))
        sched = build(counts)
        NMIX = NP - DP
        table = [u for blk in sched[2:2 + NMIX] for u in blk]

        def scope(name):
            return jax.named_scope(name) if scopes else contextlib.nullcontext()

        xa = A_x.reshape(R, D)
        xb = B_x.reshape(R, D)
        woa_t = A_wo.T
        wob_t = B_wo.T

        def body(xa_h, ka_h, va_h, wqa_h, woa_h, xb_h, kb_h, vb_h, wqb_h, wob_h, out_h,
                 x_v, wq_v, wo_v, ka_v, va_v, kb_v, vb_v, q_v, o_v, acc_v, ost_v, s_v, p_v, tab, sem):
            x_h = (xa_h, xb_h); wq_h = (wqa_h, wqb_h); wo_h = (woa_h, wob_h)

            def psplit(a):
                if isinstance(a, int):
                    return a // PPJ, a % PPJ, (a % PPJ) * 2, (a % NSP) * 2, a % NSP
                pc = a & (PPJ - 1)
                ri = a & (NSP - 1)
                return lax.shift_right_logical(a, 2), pc, pc * 2, ri * 2, ri

            def a_copies(a):
                j, _, b0, sl, ri = psplit(a)
                sm = sem.at[S_A + ri]
                return (pltpu.make_async_copy(ka_h.at[pl.ds(b0, 2), j], ka_v.at[pl.ds(sl, 2)], sm),
                        pltpu.make_async_copy(va_h.at[pl.ds(b0, 2), j], va_v.at[pl.ds(sl, 2)], sm))

            def b_copies(a):
                j, _, b0, sl, ri = psplit(a)
                sm = sem.at[S_B + ri]
                hs = pl.ds(j * rep, rep)
                return (pltpu.make_async_copy(kb_h.at[pl.ds(b0, 2), hs], kb_v.at[pl.ds(sl, 2)], sm),
                        pltpu.make_async_copy(vb_h.at[pl.ds(b0, 2), hs], vb_v.at[pl.ds(sl, 2)], sm))

            def fine_copy(k, isv):
                j, _, b0, sl, _ = psplit(NP - 1)
                src, dst = ((kb_h, kb_v), (vb_h, vb_v))[isv]
                return pltpu.make_async_copy(src.at[b0 + k, pl.ds(j * rep, rep)], dst.at[sl + k], sem.at[S_F + 2 * k + isv])

            def x_copy(br, half):
                rows = pl.ds(half * H, H)
                return pltpu.make_async_copy(x_h[br].at[rows], x_v.at[br, rows], sem.at[S_X + 2 * br + half])

            def mo(v, m):
                return v if isinstance(v, int) else pl.multiple_of(v, m)

            def wq_copy(br, j, src=None):
                cols = pl.ds(mo(j * W, W), W)
                return pltpu.make_async_copy(wq_h[br if src is None else src].at[:, cols], wq_v.at[br, j], sem.at[S_WQ + br * NJ + j])

            def wo_copy(br, j, p=None):
                cols = pl.ds(mo(j * W, W), W)
                sm = sem.at[S_WO + br * NJ + j]
                if p is None:
                    return pltpu.make_async_copy(wo_h[br].at[:, cols], wo_v.at[br, j], sm)
                rows = pl.ds(mo(p * PR, 8), PR)
                return pltpu.make_async_copy(wo_h[br].at[rows, cols], wo_v.at[br, j, rows], sm)

            def out_copy(t):
                return pltpu.make_async_copy(ost_v.at[t], out_h.at[pl.ds(t * 128, 128)], sem.at[S_OUT + t])

            def cond(pred, fn):
                if isinstance(pred, bool):
                    if pred: fn()
                else:
                    pl.when(pred)(fn)

            def issue(m):
                bb = m - DP
                def fb():
                    for c in b_copies(bb): c.start()
                def fa():
                    for c in a_copies(m): c.start()
                def fwa():
                    j, pc, _, _, _ = psplit(m)
                    wo_copy(0, j + 1, pc).start()
                def fwb():
                    j, pc, _, _, _ = psplit(bb)
                    wo_copy(1, j + 1, pc).start()
                if isinstance(m, int):
                    cond(m < NP, fa); cond(0 <= bb < NP - 1, fb); cond(m < NP - PPJ, fwa); cond(0 <= bb < NP - PPJ, fwb)
                else:
                    cond(m < NP, fa); cond(bb < NP - 1, fb); cond(m < NP - PPJ, fwa); cond(bb < NP - PPJ, fwb)

            def wait_a(a):
                def f():
                    wo_copy(0, psplit(a)[0]).wait()
                cond(psplit(a)[1] == 0, f)
                for c in a_copies(a): c.wait()

            def wait_b(a, kv=True):
                def f():
                    wo_copy(1, psplit(a)[0]).wait()
                cond(psplit(a)[1] == 0, f)
                if kv:
                    for c in b_copies(a): c.wait()

            wq_copy(0, 0).start()
            x_copy(0, 0).start()
            x_copy(0, 1).start()
            for j in range(1, NJ): wq_copy(0, j).start()
            x_copy(1, 0).start()
            x_copy(1, 1).start()
            for j in range(NJ): wq_copy(1, j).start()
            for br in range(2): wo_copy(br, 0).start()
            NP1 = (2 * NJ - 2 - 1 - 1) // p1c
            npre = L - NP1
            assert npre >= DP
            for m in range(npre): issue(m)

            for i, (br, j, t, rh) in enumerate(table):
                tab[i] = br | (j << 1) | (t << 4) | (rh << 7)
            acc_v[...] = jnp.zeros(acc_v.shape, acc_v.dtype)

            def qproj(br, j, b0, nb):
                r0 = b0 * Sq
                q = (jnp.dot(x_v[br, pl.ds(r0, nb * Sq), :], wq_v[br, j], preferred_element_type=jnp.float32) * qscale).astype(bf16)
                for bb in range(nb):
                    for h in range(rep):
                        q_v[br, j, b0 + bb, h] = q[bb * Sq:(bb + 1) * Sq, h * Dh:(h + 1) * Dh]

            with scope('S_p1a'):
                wq_copy(0, 0).wait()
                x_copy(0, 0).wait()
                qproj(0, 0, 0, B // 2)
                x_copy(0, 1).wait()
                wq_copy(0, 1).wait()
                qproj(0, 0, B // 2, B // 2)
                qproj(0, 1, 0, B)

            def p1(i, carry):
                c0 = 2 + i * p1c
                @pl.when(c0 + p1c - 1 >= NJ)
                def _():
                    pass
                @pl.when(jnp.logical_and(c0 <= NJ, c0 + p1c - 1 >= NJ))
                def _():
                    x_copy(1, 0).wait()
                    x_copy(1, 1).wait()
                cs = [(lax.shift_right_logical(c0 + k, 3), (c0 + k) & (NJ - 1)) for k in range(p1c)]
                for br, j in cs: wq_copy(br, j, src=0).wait()
                issue(npre + i)
                for br, j in cs: qproj(br, j, 0, B)
                return carry
            with scope('S_p1'):
                lax.fori_loop(0, NP1, p1, 0)

            def ounit(br, j, t, rh, nr):
                if isinstance(t, int):
                    r0, w0 = t * 128, rh * HD
                    d0 = br * D + w0
                else:
                    r0 = pl.multiple_of(t * 128, 128)
                    w0 = pl.multiple_of(rh * HD, 16)
                    d0 = pl.multiple_of(br * D + w0, 8)
                ot = o_v[br, pl.ds(r0, 128), :]
                lhs = wo_v[br, j, pl.ds(w0, nr), :]
                acc_v[t, pl.ds(d0, nr), :] += lax.dot_general(lhs, ot, NT, preferred_element_type=jnp.float32)

            def tunit(i):
                e = tab[i]
                ounit(e & 1, lax.shift_right_logical(e, 1) & 7, lax.shift_right_logical(e, 4) & 7,
                      lax.shift_right_logical(e, 7), HD)

            def sunits(us):
                us = list(us)
                while us:
                    br, j, t, rh = us.pop(0)
                    if us and rh == 0 and us[0] == (br, j, t, 1):
                        us.pop(0)
                        ounit(br, j, t, 0, D)
                    else:
                        ounit(br, j, t, rh, HD)

            def finalize(t, start=True):
                ost_v[t] = acc_v[t].T.astype(bf16)
                if start: out_copy(t).start()

            def a_item(a, k, r0):
                j, _, b0, sl, _ = psplit(a)
                return (0, j, b0 + k, sl + k, None, r0)

            def b_items(a, k, r0):
                j, _, b0, sl, _ = psplit(a)
                return [(1, j, b0 + k, sl + k, h, r0 + h * Sq) for h in range(rep)]

            def QK(items):
                res = []
                for it in items:
                    br, j, b, slot, h, r0 = it
                    if br == 0:
                        q, kk = q_v[0, j, b].reshape(rep * Sq, Dh), ka_v[slot]
                    else:
                        q, kk = q_v[1, j, b, h], kb_v[slot, h]
                    sc = lax.dot_general(q, kk, NT, preferred_element_type=jnp.float32)
                    s_v[r0:r0 + q.shape[0], :] = sc
                    res.append((it, q.shape[0], jnp.max(sc, axis=-1, keepdims=True)))
                return res

            def SM(res):
                out = []
                for it, n, m in res:
                    r0 = it[5]
                    p = jnp.exp2(s_v[r0:r0 + n, :] - m)
                    l = jnp.sum(p, axis=-1, keepdims=True)
                    p = p.astype(bf16)
                    for c in range(KC):
                        p_v[c, r0:r0 + n, :] = p[:, c * 128:(c + 1) * 128]
                    out.append((it, n, 1.0 / l))
                return out

            def PV(res):
                for it, n, r in res:
                    br, j, b, slot, h, r0 = it
                    rows = pl.ds(mo(b * Sq, 16), Sq)
                    v = va_v[slot] if br == 0 else vb_v[slot, h]
                    p = jnp.concatenate([p_v[c, r0:r0 + n, :] for c in range(KC)], axis=1)
                    o = (jnp.dot(p, v, preferred_element_type=jnp.float32) * r).astype(bf16)
                    if br == 0:
                        for hh in range(rep):
                            o_v[0, rows, hh * Dh:(hh + 1) * Dh] = o[hh * Sq:(hh + 1) * Sq]
                    else:
                        o_v[1, rows, h * Dh:(h + 1) * Dh] = o

            RA = rep * Sq
            with scope('S_pa'):
                for blk in range(2):
                    wq_copy(1, NJ - 2 + blk).wait()
                    wait_a(2 * blk); wait_a(2 * blk + 1)
                    its = [a_item(2 * blk + (i >> 1), i & 1, i * RA) for i in range(4)]
                    r01 = QK(its[:2])
                    sunits(sched[blk])
                    r23 = QK(its[2:])
                    qproj(1, NJ - 2 + blk, 0, B // 2)
                    PV(SM(r01))
                    issue(L + 2 * blk)
                    PV(SM(r23))
                    issue(L + 2 * blk + 1)
                    qproj(1, NJ - 2 + blk, B // 2, B // 2)

            def pm(n, carry):
                a = n + DP
                wait_a(a); wait_b(n)
                i0 = [a_item(a, 0, 0)] + b_items(n, 0, RA)
                i1 = [a_item(a, 1, 2 * RA)] + b_items(n, 1, 3 * RA)
                r0 = QK(i0)
                for i in range(4): tunit(n * UPB + i)
                r1 = QK(i1)
                for i in range(4, UPB): tunit(n * UPB + i)
                PV(SM(r0))
                issue(a + L)
                PV(SM(r1))
                return carry
            with scope('S_pm'):
                lax.fori_loop(0, NMIX, pm, 0)

            with scope('S_pb'):
                for k in range(2):
                    for isv in range(2): fine_copy(k, isv).start()
                ts = sched[2 + NMIX:]
                fin = 0
                for blk in range(DP - 1):
                    a = NMIX + blk
                    wait_b(a)
                    r0 = QK(b_items(a, 0, 0))
                    us = ts[blk]
                    sunits(us[:(len(us) + 2) // 4 * 2])
                    r1 = QK(b_items(a, 1, RA))
                    sunits(us[(len(us) + 2) // 4 * 2:])
                    if blk == 2:
                        finalize(0, not late_out)
                    PV(SM(r0)); PV(SM(r1))
                a = NP - 1
                fine_copy(0, 0).wait(); fine_copy(0, 1).wait()
                r0 = QK(b_items(a, 0, 0))
                sunits(ts[3])
                finalize(1, not late_out); finalize(2, not late_out)
                PV(SM(r0))
                fine_copy(1, 0).wait()
                r1 = QK(b_items(a, 1, RA))
                sunits(ts[4])
                finalize(3, not late_out); finalize(4, not late_out)
                r1 = SM(r1)
                fine_copy(1, 1).wait()
                if late_out:
                    for t in range(5): out_copy(t).start()
                PV(r1)
                finalize(5)
                sunits(ts[5])
                finalize(6)
                for t in range(NTL):
                    out_copy(t).wait()

        ms = pltpu.HBM
        out = pl.pallas_call(
            body,
            in_specs=[pl.BlockSpec(memory_space=ms)] * 10,
            out_specs=pl.BlockSpec(memory_space=ms),
            out_shape=jax.ShapeDtypeStruct((R, 2 * D), A_x.dtype),
            scratch_shapes=[
                pltpu.VMEM((2, R, D), bf16),
                pltpu.VMEM((2, NJ, D, W), bf16),
                pltpu.VMEM((2, NJ, D, W), bf16),
                pltpu.VMEM((2 * NSP, Sk, Dh), bf16),
                pltpu.VMEM((2 * NSP, Sk, Dh), bf16),
                pltpu.VMEM((2 * NSP, rep, Sk, Dh), bf16),
                pltpu.VMEM((2 * NSP, rep, Sk, Dh), bf16),
                pltpu.VMEM((2, NJ, B, rep, Sq, Dh), bf16),
                pltpu.VMEM((2, R, W), bf16),
                pltpu.VMEM((NTL, 2 * D, 128), jnp.float32),
                pltpu.VMEM((NTL, 128, 2 * D), bf16),
                pltpu.VMEM((4 * rep * Sq, Sk), jnp.float32),
                pltpu.VMEM((KC, 4 * rep * Sq, 128), bf16),
                pltpu.SMEM((len(table),), jnp.int32),
                pltpu.SemaphoreType.DMA((NSEM,)),
            ],
            compiler_params=pltpu.CompilerParams(vmem_limit_bytes=120 * 1024 * 1024,
                                                 disable_bounds_checks=True, disable_semaphore_checks=True),
        )(xa, A_k_cache, A_v_cache, A_wq, woa_t, xb, B_k_cache, B_v_cache, B_wq, wob_t)
        return out.reshape(B, Sq, 2 * D)
    return kernel


_impl = make(L=10,late_out=False)


@jax.jit
def pallas_concat_heads__gqa_block_cached__mha_block_cached__near_ridge_kernel(A_x, A_k_cache, A_v_cache, A_wq, A_wo, B_x, B_k_cache, B_v_cache, B_wq, B_wo):
    return _impl(A_x, A_k_cache, A_v_cache, A_wq, A_wo, B_x, B_k_cache, B_v_cache, B_wq, B_wo)
```

```python
import jax
import jax.numpy as jnp
from jax import lax
import jax.experimental.pallas as pl
import jax.experimental.pallas.tpu as pltpu

_LOG2E = 1.4426950408889634
_NT = (((1,), (1,)), ((), ()))

_HQ, _DH = 16, 256
_L = 10
_DP = 4
_P1C = 2
_NSP = 16
_UPB = 7
_OUT_STAGE = (2, 2, 2, 2, 3, 4)
_NSPLIT = 2


def _schedule(B, NJ, NTL, DP, last_pa):
    NP, NST, NQ = NJ * B // 2, NJ * B, DP // 2
    NMIX = NP - DP
    blocks = [(-1 if k < NQ - 1 else last_pa, 4 * k, 0, 4 * k + 4, 0) for k in range(NQ)]
    blocks += [(_UPB, 2 * (m + DP), 2 * m, 2 * (m + DP + 1), 2 * (m + 1)) for m in range(NMIX)]
    blocks += [(-1, NST, 2 * m, NST, 2 * m + 2) for m in range(NMIX, NP - 2)]
    blocks += [(-1, NST, s, NST, min(s + 1, NST - 1)) for s in range(NST - 4, NST)]
    blocks += [(-1, NST, NST, NST, NST)]
    queue, pushed, out = [], [0, 0], []
    for n, da, db, ea, eb in blocks:
        for br, done in ((0, da), (1, db)):
            ready = (done // B) * NTL + max(0, done % B - 1)
            while pushed[br] < ready:
                j, t = divmod(pushed[br], NTL)
                pushed[br] += 1
                queue += [(br, j, t, 0), (br, j, t, 1)]
        queue.sort(key=lambda u: (u[1] * B + u[2] - (2 * DP if u[0] == 0 else 0), u[0], u[3]))
        if n < 0:
            n = len(queue)
        if len(queue) < n:
            return None
        out.append(queue[:n])
        queue = queue[n:]
        if any((ea, eb)[br] > (j + 1) * B + t for br, j, t, _ in queue):
            return None
    assert not queue and pushed == [NJ * NTL] * 2
    return out


@jax.jit
def pallas_concat_heads__gqa_block_cached__mha_block_cached__near_ridge_kernel(
    A_x: jax.Array,
    A_k_cache: jax.Array,
    A_v_cache: jax.Array,
    A_wq: jax.Array,
    A_wo: jax.Array,
    B_x: jax.Array,
    B_k_cache: jax.Array,
    B_v_cache: jax.Array,
    B_wq: jax.Array,
    B_wo: jax.Array,
):
    B, Sq, D = A_x.shape
    Dh = _DH
    NJ, Sk = A_k_cache.shape[1], A_k_cache.shape[2]
    rep = _HQ // NJ
    W = rep * Dh
    R = B * Sq
    NTL = R // 128
    PPJ = B // 2
    NP = NJ * PPJ
    NST = NJ * B
    L, DP, NSP, UPB = _L, _DP, _NSP, _UPB
    NQ = DP // 2
    NMIX = NP - DP
    HD = D // 2
    KC = Sk // 128
    RA = rep * Sq
    CA = D // 128 * 128
    X0 = B // 2
    assert (B, NJ, rep, NTL) == (8, 8, 2, 7) and R == NTL * 128 and Sq % 16 == 0 and HD % 16 == 0
    assert B_k_cache.shape[1] == _HQ and DP <= L < NSP - 1
    qscale = Dh ** -0.5 * _LOG2E
    bf16, f32 = jnp.bfloat16, jnp.float32

    S_X = 0
    S_WQ = S_X + 3
    S_WO = S_WQ + 4
    S_A = S_WO + 1
    S_B = S_A + NSP
    S_F = S_B + NSP
    S_OUT = S_F + 5
    NSEM = S_OUT + 2 * NTL

    sched = next(s for s in (_schedule(B, NJ, NTL, DP, n) for n in range(2 * NTL, -1, -1)) if s is not None)
    table = [u for blk in sched[NQ:NQ + NMIX] for u in blk]
    tail = sched[NQ + NMIX:]

    def body(xa_h, ka_h, va_h, wqa_h, woa_h, xb_h, kb_h, vb_h, wqb_h, wob_h, out_h,
             x_v, wq_v, wo_v, ka_v, va_v, kb_v, vb_v, q_v, o_v, acc_v, ost_v, s_v, p_v, tab, sem):

        def mo(v, m):
            return v if isinstance(v, int) else pl.multiple_of(v, m)

        def shr(v, n):
            return v >> n if isinstance(v, int) else lax.shift_right_logical(v, n)

        def psplit(a):
            ri = a & (NSP - 1)
            return shr(a, 2), (a & (PPJ - 1)) * 2, ri * 2, ri

        def a_copies(a):
            j, b0, sl, ri = psplit(a)
            sm = sem.at[S_A + ri]
            return (pltpu.make_async_copy(ka_h.at[pl.ds(b0, 2), j], ka_v.at[pl.ds(sl, 2)], sm),
                    pltpu.make_async_copy(va_h.at[pl.ds(b0, 2), j], va_v.at[pl.ds(sl, 2)], sm))

        def b_copies(a):
            j, b0, sl, ri = psplit(a)
            sm = sem.at[S_B + ri]
            hs = pl.ds(j * rep, rep)
            return (pltpu.make_async_copy(kb_h.at[pl.ds(b0, 2), hs], kb_v.at[pl.ds(sl, 2)], sm),
                    pltpu.make_async_copy(vb_h.at[pl.ds(b0, 2), hs], vb_v.at[pl.ds(sl, 2)], sm))

        def fine_copy(st, isv):
            j, b0, sl, _ = psplit(st // 2)
            src, dst = ((kb_h, kb_v), (vb_h, vb_v))[isv]
            si = st - (NST - 4) + (isv if st == NST - 1 else 0)
            return pltpu.make_async_copy(src.at[b0 + st % 2, pl.ds(j * rep, rep)], dst.at[sl + st % 2],
                                         sem.at[S_F + si])

        def x_copy(i):
            src, br, r0, r1 = ((xa_h, 0, 0, X0 * Sq), (xa_h, 0, X0 * Sq, R), (xb_h, 1, 0, R))[i]
            return pltpu.make_async_copy(src.at[r0:r1], x_v.at[br, r0:r1], sem.at[S_X + i])

        def wq_copy(i):
            src, br, c0, c1 = ((wqa_h, 0, 0, W), (wqa_h, 0, W, 2 * W), (wqa_h, 0, 2 * W, NJ * W),
                               (wqb_h, 1, 0, NJ * W))[i]
            return pltpu.make_async_copy(src.at[:, c0:c1], wq_v.at[br, :, c0:c1], sem.at[S_WQ + i])

        def wo_copy(br):
            return pltpu.make_async_copy((woa_h, wob_h)[br], wo_v.at[br], sem.at[S_WO])

        def cols(part):
            return {None: (0, 2 * D), 0: (0, CA), 1: (CA, 2 * D)}[part]

        def out_copy(t, part):
            c0, c1 = cols(part)
            return pltpu.make_async_copy(ost_v.at[t, :, c0:c1], out_h.at[t * 128:(t + 1) * 128, c0:c1],
                                         sem.at[S_OUT + t + (NTL if part == 0 else 0)])

        def issue(m):
            def start_a():
                for c in a_copies(m):
                    c.start()

            def start_b():
                for c in b_copies(m - DP):
                    c.start()

            if isinstance(m, int):
                if m < NP:
                    start_a()
                if 0 <= m - DP < NP - 2:
                    start_b()
            else:
                pl.when(m < NP)(start_a)
                pl.when(m - DP < NP - 2)(start_b)

        def wait_a(a):
            for c in a_copies(a):
                c.wait()

        def wait_b(a):
            for c in b_copies(a):
                c.wait()

        def qproj(br, j, b0, nb):
            x = x_v[br, b0 * Sq:(b0 + nb) * Sq, :]
            q = jnp.dot(x, wq_v[br, :, pl.ds(mo(j * W, W), W)], preferred_element_type=f32)
            q = (q * qscale).astype(bf16)
            for bb in range(nb):
                for h in range(rep):
                    q_v[br, j, b0 + bb, h] = q[bb * Sq:(bb + 1) * Sq, h * Dh:(h + 1) * Dh]

        def ounit(br, j, t, rh, nr):
            w0 = mo(rh * HD, 16)
            ot = o_v[br, pl.ds(mo(t * 128, 128), 128), :]
            lhs = wo_v[br, pl.ds(w0, nr), pl.ds(mo(j * W, W), W)]
            acc_v[t, pl.ds(mo(br * D + w0, 8), nr), :] += lax.dot_general(lhs, ot, _NT, preferred_element_type=f32)

        def table_unit(i):
            e = tab[i]
            ounit(e & 1, shr(e, 1) & 7, shr(e, 4) & 7, shr(e, 7), HD)

        def static_units(us):
            us = list(us)
            while us:
                br, j, t, rh = us.pop(0)
                if us and rh == 0 and us[0] == (br, j, t, 1):
                    us.pop(0)
                    ounit(br, j, t, 0, D)
                else:
                    ounit(br, j, t, rh, HD)

        def finalize(t, part):
            c0, c1 = cols(part)
            ost_v[t, :, c0:c1] = acc_v[t, c0:c1, :].T.astype(ost_v.dtype)

        def a_item(a, k, r0):
            j, b0, sl, _ = psplit(a)
            return (0, j, b0 + k, sl + k, None, r0)

        def b_items(a, k, r0):
            j, b0, sl, _ = psplit(a)
            return [(1, j, b0 + k, sl + k, h, r0 + h * Sq) for h in range(rep)]

        def scores(items):
            res = []
            for it in items:
                br, j, b, slot, h, r0 = it
                if br == 0:
                    q, k = q_v[0, j, b].reshape(RA, Dh), ka_v[slot]
                else:
                    q, k = q_v[1, j, b, h], kb_v[slot, h]
                s = lax.dot_general(q, k, _NT, preferred_element_type=f32)
                s_v[r0:r0 + q.shape[0], :] = s
                res.append((it, q.shape[0], jnp.max(s, axis=-1, keepdims=True)))
            return res

        def softmax(res):
            out = []
            for it, n, m in res:
                r0 = it[5]
                p = jnp.exp2(s_v[r0:r0 + n, :] - m)
                denom = jnp.sum(p, axis=-1, keepdims=True)
                p = p.astype(bf16)
                for c in range(KC):
                    p_v[c, r0:r0 + n, :] = p[:, c * 128:(c + 1) * 128]
                out.append((it, n, 1.0 / denom))
            return out

        def values(res):
            for it, n, rinv in res:
                br, j, b, slot, h, r0 = it
                rows = pl.ds(mo(b * Sq, 16), Sq)
                v = va_v[slot] if br == 0 else vb_v[slot, h]
                p = jnp.concatenate([p_v[c, r0:r0 + n, :] for c in range(KC)], axis=1)
                o = (jnp.dot(p, v, preferred_element_type=f32) * rinv).astype(bf16)
                if br == 0:
                    for hh in range(rep):
                        o_v[0, rows, hh * Dh:(hh + 1) * Dh] = o[hh * Sq:(hh + 1) * Sq]
                else:
                    o_v[1, rows, h * Dh:(h + 1) * Dh] = o

        for c in (wq_copy(0), x_copy(0), x_copy(1), wq_copy(1), wq_copy(2), x_copy(2), wq_copy(3),
                  wo_copy(0), wo_copy(1)):
            c.start()
        for m in range(L):
            issue(m)
        for i, (br, j, t, rh) in enumerate(table):
            tab[i] = br | (j << 1) | (t << 4) | (rh << 7)
        acc_v[...] = jnp.zeros(acc_v.shape, acc_v.dtype)

        nch = 2 * NJ - NQ
        n_it = (nch - 2) // _P1C
        c_first = nch - n_it * _P1C
        wq_copy(0).wait()
        x_copy(0).wait()
        qproj(0, 0, 0, X0)
        x_copy(1).wait()
        wq_copy(1).wait()
        qproj(0, 0, X0, B - X0)
        qproj(0, 1, 0, B)
        wq_copy(2).wait()
        for c in range(2, c_first):
            qproj(0, c, 0, B)

        def qproj_step(i, carry):
            c0 = c_first + i * _P1C

            @pl.when(jnp.logical_and(c0 <= NJ, c0 + _P1C > NJ))
            def _():
                x_copy(2).wait()
                wq_copy(3).wait()

            for k in range(_P1C):
                qproj(shr(c0 + k, 3), (c0 + k) & (NJ - 1), 0, B)
            return carry

        lax.fori_loop(0, n_it, qproj_step, 0)

        for br in range(2):
            wo_copy(br).wait()
        for blk in range(NQ):
            jq = NJ - NQ + blk
            wait_a(2 * blk)
            wait_a(2 * blk + 1)
            its = [a_item(2 * blk + (i >> 1), i & 1, i * RA) for i in range(4)]
            s01 = scores(its[:2])
            static_units(sched[blk])
            s23 = scores(its[2:])
            qproj(1, jq, 0, B // 2)
            values(softmax(s01))
            issue(L + 2 * blk)
            values(softmax(s23))
            issue(L + 2 * blk + 1)
            qproj(1, jq, B // 2, B // 2)

        def mixed(n, carry):
            a = n + DP
            wait_a(a)
            wait_b(n)
            s0 = scores([a_item(a, 0, 0)] + b_items(n, 0, RA))
            for i in range(4):
                table_unit(n * UPB + i)
            s1 = scores([a_item(a, 1, 2 * RA)] + b_items(n, 1, 3 * RA))
            for i in range(4, UPB):
                table_unit(n * UPB + i)
            values(softmax(s0))
            issue(a + L)
            values(softmax(s1))
            return carry

        lax.fori_loop(0, NMIX, mixed, 0)

        for st in range(NST - 4, NST):
            for isv in range(2):
                fine_copy(st, isv).start()
        for blk in range(DP - 2):
            a = NMIX + blk
            wait_b(a)
            us = tail[blk]
            cut = (len(us) + 2) // 4 * 2
            s0 = scores(b_items(a, 0, 0))
            static_units(us[:cut])
            s1 = scores(b_items(a, 1, RA))
            static_units(us[cut:])
            values(softmax(s0))
            values(softmax(s1))

        fine = tail[DP - 2:]
        done_at = {t: -1 for t in range(NTL)}
        for si, us in enumerate(fine):
            for br, j, t, _ in us:
                assert br == 1 and j == NJ - 1
                done_at[t] = si
        split = range(NTL - _NSPLIT, NTL)

        def part(t):
            return 1 if t in split else None

        def flush(si):
            if si == 0:
                for t in split:
                    finalize(t, 0)
            for t in range(NTL - 1):
                if done_at[t] + 1 == si:
                    finalize(t, part(t))
            for t in range(NTL - 1):
                assert _OUT_STAGE[t] > done_at[t]
                if _OUT_STAGE[t] == si:
                    out_copy(t, part(t)).start()
            if si == 0:
                for t in split:
                    out_copy(t, 0).start()

        for si in range(3):
            st = NST - 4 + si
            fine_copy(st, 0).wait()
            fine_copy(st, 1).wait()
            s0 = scores(b_items(st // 2, st % 2, 0))
            static_units(fine[si])
            flush(si)
            values(softmax(s0))
        st = NST - 1
        fine_copy(st, 0).wait()
        s0 = scores(b_items(st // 2, st % 2, 0))
        static_units(fine[3])
        flush(3)
        p0 = softmax(s0)
        fine_copy(st, 1).wait()
        values(p0)
        flush(4)
        static_units(fine[4])
        finalize(NTL - 1, part(NTL - 1))
        out_copy(NTL - 1, part(NTL - 1)).start()
        for t in range(NTL):
            out_copy(t, part(t)).wait()
        for t in split:
            out_copy(t, 0).wait()

    hbm = pl.BlockSpec(memory_space=pltpu.HBM)
    out = pl.pallas_call(
        body,
        in_specs=[hbm] * 10,
        out_specs=hbm,
        out_shape=jax.ShapeDtypeStruct((R, 2 * D), A_x.dtype),
        scratch_shapes=[
            pltpu.VMEM((2, R, D), bf16),
            pltpu.VMEM((2, D, NJ * W), bf16),
            pltpu.VMEM((2, D, NJ * W), bf16),
            pltpu.VMEM((2 * NSP, Sk, Dh), bf16),
            pltpu.VMEM((2 * NSP, Sk, Dh), bf16),
            pltpu.VMEM((2 * NSP, rep, Sk, Dh), bf16),
            pltpu.VMEM((2 * NSP, rep, Sk, Dh), bf16),
            pltpu.VMEM((2, NJ, B, rep, Sq, Dh), bf16),
            pltpu.VMEM((2, R, W), bf16),
            pltpu.VMEM((NTL, 2 * D, 128), f32),
            pltpu.VMEM((NTL, 128, 2 * D), A_x.dtype),
            pltpu.VMEM((4 * RA, Sk), f32),
            pltpu.VMEM((KC, 4 * RA, 128), bf16),
            pltpu.SMEM((len(table),), jnp.int32),
            pltpu.SemaphoreType.DMA((NSEM,)),
        ],
        compiler_params=pltpu.CompilerParams(
            vmem_limit_bytes=120 * 1024 * 1024,
            disable_bounds_checks=True,
            disable_semaphore_checks=True,
        ),
    )(A_x.reshape(R, D), A_k_cache, A_v_cache, A_wq, A_wo.T,
      B_x.reshape(R, D), B_k_cache, B_v_cache, B_wq, B_wo.T)
    return out.reshape(B, Sq, 2 * D)
```

```python
import jax
import jax.numpy as jnp
from jax import lax
import jax.experimental.pallas as pl
import jax.experimental.pallas.tpu as pltpu

_NT = (((1,), (1,)), ((), ()))

_HQ, _DH = 16, 256
_L = 10
_DP = 4
_P1C = 4
_NSP = 16
_UPB = 7
_OUT_STAGE = (2, 2, 2, 2, 3, 4)
_NSPLIT = 2


def _schedule(B, NJ, NTL, DP, last_pa):
    NP, NST, NQ = NJ * B // 2, NJ * B, DP // 2
    NMIX = NP - DP
    blocks = [(-1 if k < NQ - 1 else last_pa, 4 * k, 0, 4 * k + 4, 0) for k in range(NQ)]
    blocks += [(_UPB, 2 * (m + DP), 2 * m, 2 * (m + DP + 1), 2 * (m + 1)) for m in range(NMIX)]
    blocks += [(-1, NST, 2 * m, NST, 2 * m + 2) for m in range(NMIX, NP - 2)]
    blocks += [(-1, NST, s, NST, min(s + 1, NST - 1)) for s in range(NST - 4, NST)]
    blocks += [(-1, NST, NST, NST, NST)]
    queue, pushed, out = [], [0, 0], []
    for n, da, db, ea, eb in blocks:
        for br, done in ((0, da), (1, db)):
            ready = (done // B) * NTL + max(0, done % B - 1)
            while pushed[br] < ready:
                j, t = divmod(pushed[br], NTL)
                pushed[br] += 1
                queue += [(br, j, t, 0), (br, j, t, 1)]
        queue.sort(key=lambda u: (u[1] * B + u[2] - (2 * DP if u[0] == 0 else 0), u[0], u[3]))
        if n < 0:
            n = len(queue)
        if len(queue) < n:
            return None
        out.append(queue[:n])
        queue = queue[n:]
        if any((ea, eb)[br] > (j + 1) * B + t for br, j, t, _ in queue):
            return None
    assert not queue and pushed == [NJ * NTL] * 2
    return out


@jax.jit
def pallas_concat_heads__gqa_block_cached__mha_block_cached__near_ridge_kernel(
    A_x: jax.Array,
    A_k_cache: jax.Array,
    A_v_cache: jax.Array,
    A_wq: jax.Array,
    A_wo: jax.Array,
    B_x: jax.Array,
    B_k_cache: jax.Array,
    B_v_cache: jax.Array,
    B_wq: jax.Array,
    B_wo: jax.Array,
):
    B, Sq, D = A_x.shape
    Dh = _DH
    NJ, Sk = A_k_cache.shape[1], A_k_cache.shape[2]
    rep = _HQ // NJ
    W = rep * Dh
    R = B * Sq
    NTL = R // 128
    PPJ = B // 2
    NP = NJ * PPJ
    NST = NJ * B
    L, DP, NSP, UPB = _L, _DP, _NSP, _UPB
    NQ = DP // 2
    NMIX = NP - DP
    HD = D // 2
    KC = Sk // 128
    RA = rep * Sq
    CA = D // 128 * 128
    X0 = B // 2
    assert (B, NJ, rep, NTL) == (8, 8, 2, 7) and R == NTL * 128 and Sq % 16 == 0 and HD % 16 == 0
    assert B_k_cache.shape[1] == _HQ and DP <= L < NSP - 1
    qscale = Dh ** -0.5
    bf16, f32 = jnp.bfloat16, jnp.float32

    S_X = 0
    S_WQ = S_X + 3
    S_WO = S_WQ + 4
    S_A = S_WO + 1
    S_B = S_A + NSP
    S_F = S_B + NSP
    S_OUT = S_F + 5
    NSEM = S_OUT + 2 * NTL

    sched = next(s for s in (_schedule(B, NJ, NTL, DP, n) for n in range(2 * NTL, -1, -1)) if s is not None)
    table = [u for blk in sched[NQ:NQ + NMIX] for u in blk]
    tail = sched[NQ + NMIX:]

    def body(xa_h, ka_h, va_h, wqa_h, woa_h, xb_h, kb_h, vb_h, wqb_h, wob_h, out_h,
             x_v, wq_v, wo_v, ka_v, va_v, kb_v, vb_v, q_v, o_v, acc_v, ost_v, s_v, p_v, tab, sem):

        def mo(v, m):
            return v if isinstance(v, int) else pl.multiple_of(v, m)

        def shr(v, n):
            return v >> n if isinstance(v, int) else lax.shift_right_logical(v, n)

        def psplit(a):
            ri = a & (NSP - 1)
            return shr(a, 2), (a & (PPJ - 1)) * 2, ri * 2, ri

        def a_copies(a):
            j, b0, sl, ri = psplit(a)
            sm = sem.at[S_A + ri]
            return (pltpu.make_async_copy(ka_h.at[pl.ds(b0, 2), j], ka_v.at[pl.ds(sl, 2)], sm),
                    pltpu.make_async_copy(va_h.at[pl.ds(b0, 2), j], va_v.at[pl.ds(sl, 2)], sm))

        def b_copies(a):
            j, b0, sl, ri = psplit(a)
            sm = sem.at[S_B + ri]
            hs = pl.ds(j * rep, rep)
            return (pltpu.make_async_copy(kb_h.at[pl.ds(b0, 2), hs], kb_v.at[pl.ds(sl, 2)], sm),
                    pltpu.make_async_copy(vb_h.at[pl.ds(b0, 2), hs], vb_v.at[pl.ds(sl, 2)], sm))

        def fine_copy(st, isv):
            j, b0, sl, _ = psplit(st // 2)
            src, dst = ((kb_h, kb_v), (vb_h, vb_v))[isv]
            si = st - (NST - 4) + (isv if st == NST - 1 else 0)
            return pltpu.make_async_copy(src.at[b0 + st % 2, pl.ds(j * rep, rep)], dst.at[sl + st % 2],
                                         sem.at[S_F + si])

        def x_copy(i):
            src, br, r0, r1 = ((xa_h, 0, 0, X0 * Sq), (xa_h, 0, X0 * Sq, R), (xb_h, 1, 0, R))[i]
            return pltpu.make_async_copy(src.at[r0:r1], x_v.at[br, r0:r1], sem.at[S_X + i])

        def wq_copy(i):
            src, br, c0, c1 = ((wqa_h, 0, 0, W), (wqa_h, 0, W, 2 * W), (wqa_h, 0, 2 * W, NJ * W),
                               (wqb_h, 1, 0, NJ * W))[i]
            return pltpu.make_async_copy(src.at[:, c0:c1], wq_v.at[br, :, c0:c1], sem.at[S_WQ + i])

        def wo_copy(br):
            return pltpu.make_async_copy((woa_h, wob_h)[br], wo_v.at[br], sem.at[S_WO])

        def cols(part):
            return {None: (0, 2 * D), 0: (0, CA), 1: (CA, 2 * D)}[part]

        def out_copy(t, part):
            c0, c1 = cols(part)
            return pltpu.make_async_copy(ost_v.at[t, :, c0:c1], out_h.at[t * 128:(t + 1) * 128, c0:c1],
                                         sem.at[S_OUT + t + (NTL if part == 0 else 0)])

        def issue(m):
            def start_a():
                for c in a_copies(m):
                    c.start()

            def start_b():
                for c in b_copies(m - DP):
                    c.start()

            if isinstance(m, int):
                if m < NP:
                    start_a()
                if 0 <= m - DP < NP - 2:
                    start_b()
            else:
                pl.when(m < NP)(start_a)
                pl.when(m - DP < NP - 2)(start_b)

        def wait_a(a):
            for c in a_copies(a):
                c.wait()

        def wait_b(a):
            for c in b_copies(a):
                c.wait()

        def qproj(br, j, b0, nb):
            x = x_v[br, b0 * Sq:(b0 + nb) * Sq, :]
            q = jnp.dot(x, wq_v[br, :, pl.ds(mo(j * W, W), W)], preferred_element_type=f32)
            q = (q * qscale).astype(bf16)
            for bb in range(nb):
                for h in range(rep):
                    q_v[br, j, b0 + bb, h] = q[bb * Sq:(bb + 1) * Sq, h * Dh:(h + 1) * Dh]

        def ounit(br, j, t, rh, nr):
            w0 = mo(rh * HD, 16)
            ot = o_v[br, pl.ds(mo(t * 128, 128), 128), :]
            lhs = wo_v[br, pl.ds(w0, nr), pl.ds(mo(j * W, W), W)]
            acc_v[t, pl.ds(mo(br * D + w0, 8), nr), :] += lax.dot_general(lhs, ot, _NT, preferred_element_type=f32)

        def table_unit(i):
            e = tab[i]
            ounit(e & 1, shr(e, 1) & 7, shr(e, 4) & 7, shr(e, 7), HD)

        def static_units(us):
            us = list(us)
            while us:
                br, j, t, rh = us.pop(0)
                if us and rh == 0 and us[0] == (br, j, t, 1):
                    us.pop(0)
                    ounit(br, j, t, 0, D)
                else:
                    ounit(br, j, t, rh, HD)

        def finalize(t, part):
            c0, c1 = cols(part)
            ost_v[t, :, c0:c1] = acc_v[t, c0:c1, :].T.astype(ost_v.dtype)

        def a_item(a, k, r0):
            j, b0, sl, _ = psplit(a)
            return (0, j, b0 + k, sl + k, None, r0)

        def b_items(a, k, r0):
            j, b0, sl, _ = psplit(a)
            return [(1, j, b0 + k, sl + k, h, r0 + h * Sq) for h in range(rep)]

        def scores(items):
            res = []
            for it in items:
                br, j, b, slot, h, r0 = it
                if br == 0:
                    q, k = q_v[0, j, b].reshape(RA, Dh), ka_v[slot]
                else:
                    q, k = q_v[1, j, b, h], kb_v[slot, h]
                s = lax.dot_general(q, k, _NT, preferred_element_type=f32)
                s_v[r0:r0 + q.shape[0], :] = s.astype(bf16).astype(f32)
                m = jnp.max(s, axis=-1, keepdims=True).astype(bf16).astype(f32)
                res.append((it, q.shape[0], m))
            return res

        def softmax(res):
            out = []
            for it, n, m in res:
                r0 = it[5]
                p = jnp.exp(s_v[r0:r0 + n, :] - m)
                denom = jnp.sum(p, axis=-1, keepdims=True)
                p = p.astype(bf16)
                for c in range(KC):
                    p_v[c, r0:r0 + n, :] = p[:, c * 128:(c + 1) * 128]
                out.append((it, n, 1.0 / denom))
            return out

        def values(res):
            for it, n, rinv in res:
                br, j, b, slot, h, r0 = it
                rows = pl.ds(mo(b * Sq, 16), Sq)
                v = va_v[slot] if br == 0 else vb_v[slot, h]
                p = jnp.concatenate([p_v[c, r0:r0 + n, :] for c in range(KC)], axis=1)
                o = (jnp.dot(p, v, preferred_element_type=f32) * rinv).astype(bf16)
                if br == 0:
                    for hh in range(rep):
                        o_v[0, rows, hh * Dh:(hh + 1) * Dh] = o[hh * Sq:(hh + 1) * Sq]
                else:
                    o_v[1, rows, h * Dh:(h + 1) * Dh] = o

        for c in (wq_copy(0), x_copy(0), x_copy(1), wq_copy(1), wq_copy(2), x_copy(2), wq_copy(3),
                  wo_copy(0), wo_copy(1)):
            c.start()
        for m in range(L):
            issue(m)
        for i, (br, j, t, rh) in enumerate(table):
            tab[i] = br | (j << 1) | (t << 4) | (rh << 7)
        acc_v[...] = jnp.zeros(acc_v.shape, acc_v.dtype)

        nch = 2 * NJ - NQ
        n_it = (nch - 2) // _P1C
        c_first = nch - n_it * _P1C
        wq_copy(0).wait()
        x_copy(0).wait()
        qproj(0, 0, 0, X0)
        x_copy(1).wait()
        wq_copy(1).wait()
        qproj(0, 0, X0, B - X0)
        qproj(0, 1, 0, B)
        wq_copy(2).wait()
        for c in range(2, c_first):
            qproj(0, c, 0, B)

        def qproj_step(i, carry):
            c0 = c_first + i * _P1C

            @pl.when(jnp.logical_and(c0 <= NJ, c0 + _P1C > NJ))
            def _():
                x_copy(2).wait()
                wq_copy(3).wait()

            for k in range(_P1C):
                qproj(shr(c0 + k, 3), (c0 + k) & (NJ - 1), 0, B)
            return carry

        lax.fori_loop(0, n_it, qproj_step, 0)

        for br in range(2):
            wo_copy(br).wait()
        for blk in range(NQ):
            jq = NJ - NQ + blk
            wait_a(2 * blk)
            wait_a(2 * blk + 1)
            its = [a_item(2 * blk + (i >> 1), i & 1, i * RA) for i in range(4)]
            s01 = scores(its[:2])
            static_units(sched[blk])
            s23 = scores(its[2:])
            qproj(1, jq, 0, B // 2)
            values(softmax(s01))
            issue(L + 2 * blk)
            values(softmax(s23))
            issue(L + 2 * blk + 1)
            qproj(1, jq, B // 2, B // 2)

        def mixed(n, carry):
            a = n + DP
            wait_a(a)
            wait_b(n)
            s0 = scores([a_item(a, 0, 0)])
            table_unit(n * UPB)
            s0 += scores(b_items(n, 0, RA))
            for i in range(1, 3):
                table_unit(n * UPB + i)
            s1 = scores([a_item(a, 1, 2 * RA)])
            table_unit(n * UPB + 3)
            s1 += scores(b_items(n, 1, 3 * RA))
            for i in range(4, UPB):
                table_unit(n * UPB + i)
            values(softmax(s0))
            issue(a + L)
            values(softmax(s1))
            return carry

        lax.fori_loop(0, NMIX, mixed, 0)

        for st in range(NST - 4, NST):
            for isv in range(2):
                fine_copy(st, isv).start()
        for blk in range(DP - 2):
            a = NMIX + blk
            wait_b(a)
            us = tail[blk]
            cut = (len(us) + 2) // 4 * 2
            s0 = scores(b_items(a, 0, 0))
            static_units(us[:cut])
            s1 = scores(b_items(a, 1, RA))
            static_units(us[cut:])
            values(softmax(s0))
            values(softmax(s1))

        fine = tail[DP - 2:]
        done_at = {t: -1 for t in range(NTL)}
        for si, us in enumerate(fine):
            for br, j, t, _ in us:
                assert br == 1 and j == NJ - 1
                done_at[t] = si
        split = range(NTL - _NSPLIT, NTL)

        def part(t):
            return 1 if t in split else None

        def flush(si):
            if si == 0:
                for t in split:
                    finalize(t, 0)
            for t in range(NTL - 1):
                if done_at[t] + 1 == si:
                    finalize(t, part(t))
            for t in range(NTL - 1):
                assert _OUT_STAGE[t] > done_at[t]
                if _OUT_STAGE[t] == si:
                    out_copy(t, part(t)).start()
            if si == 0:
                for t in split:
                    out_copy(t, 0).start()

        for si in range(3):
            st = NST - 4 + si
            fine_copy(st, 0).wait()
            fine_copy(st, 1).wait()
            s0 = scores(b_items(st // 2, st % 2, 0))
            static_units(fine[si])
            flush(si)
            values(softmax(s0))
        st = NST - 1
        fine_copy(st, 0).wait()
        s0 = scores(b_items(st // 2, st % 2, 0))
        static_units(fine[3])
        flush(3)
        p0 = softmax(s0)
        fine_copy(st, 1).wait()
        values(p0)
        flush(4)
        static_units(fine[4])
        finalize(NTL - 1, part(NTL - 1))
        out_copy(NTL - 1, part(NTL - 1)).start()
        for t in range(NTL):
            out_copy(t, part(t)).wait()
        for t in split:
            out_copy(t, 0).wait()

    hbm = pl.BlockSpec(memory_space=pltpu.HBM)
    out = pl.pallas_call(
        body,
        in_specs=[hbm] * 10,
        out_specs=hbm,
        out_shape=jax.ShapeDtypeStruct((R, 2 * D), A_x.dtype),
        scratch_shapes=[
            pltpu.VMEM((2, R, D), bf16),
            pltpu.VMEM((2, D, NJ * W), bf16),
            pltpu.VMEM((2, D, NJ * W), bf16),
            pltpu.VMEM((2 * NSP, Sk, Dh), bf16),
            pltpu.VMEM((2 * NSP, Sk, Dh), bf16),
            pltpu.VMEM((2 * NSP, rep, Sk, Dh), bf16),
            pltpu.VMEM((2 * NSP, rep, Sk, Dh), bf16),
            pltpu.VMEM((2, NJ, B, rep, Sq, Dh), bf16),
            pltpu.VMEM((2, R, W), bf16),
            pltpu.VMEM((NTL, 2 * D, 128), f32),
            pltpu.VMEM((NTL, 128, 2 * D), A_x.dtype),
            pltpu.VMEM((4 * RA, Sk), f32),
            pltpu.VMEM((KC, 4 * RA, 128), bf16),
            pltpu.SMEM((len(table),), jnp.int32),
            pltpu.SemaphoreType.DMA((NSEM,)),
        ],
        compiler_params=pltpu.CompilerParams(
            vmem_limit_bytes=120 * 1024 * 1024,
            disable_bounds_checks=True,
            disable_semaphore_checks=True,
        ),
    )(A_x.reshape(R, D), A_k_cache, A_v_cache, A_wq, A_wo.T,
      B_x.reshape(R, D), B_k_cache, B_v_cache, B_wq, B_wo.T)
    return out.reshape(B, Sq, 2 * D)
```

```python
import jax
import jax.numpy as jnp
from jax import lax
import jax.experimental.pallas as pl
import jax.experimental.pallas.tpu as pltpu

_NT = (((1,), (1,)), ((), ()))

_HQ, _DH = 16, 256
_L = 10
_DP = 4
_P1C = 4
_NSP = 16
_UPB = 7
_OUT_STAGE = (2, 2, 2, 2, 3, 4)
_NSPLIT = 2


def _schedule(B, NJ, NTL, DP, last_pa):
    NP, NST, NQ = NJ * B // 2, NJ * B, DP // 2
    NMIX = NP - DP - 1
    blocks = [(-1 if k < NQ - 1 else last_pa, 4 * k, 0, 4 * k + 4, 0) for k in range(NQ)]
    blocks += [(_UPB, 2 * (m + DP), 2 * m, 2 * (m + DP + 1), 2 * (m + 1)) for m in range(NMIX)]
    blocks += [(-1, NST - 2, 2 * NMIX, NST, 2 * NMIX)]
    blocks += [(-1, NST, 2 * m, NST, 2 * m + 2) for m in range(NMIX, NP - 2)]
    blocks += [(-1, NST, s, NST, min(s + 1, NST - 1)) for s in range(NST - 4, NST)]
    blocks += [(-1, NST, NST, NST, NST)]
    queue, pushed, out = [], [0, 0], []
    for n, da, db, ea, eb in blocks:
        for br, done in ((0, da), (1, db)):
            ready = (done // B) * NTL + max(0, done % B - 1)
            while pushed[br] < ready:
                j, t = divmod(pushed[br], NTL)
                pushed[br] += 1
                queue += [(br, j, t, 0), (br, j, t, 1)]
        queue.sort(key=lambda u: (u[1] * B + u[2] - (2 * DP if u[0] == 0 else 0), u[0], u[3]))
        if n < 0:
            n = len(queue)
        if len(queue) < n:
            return None
        out.append(queue[:n])
        queue = queue[n:]
        if any((ea, eb)[br] > (j + 1) * B + t for br, j, t, _ in queue):
            return None
    assert not queue and pushed == [NJ * NTL] * 2
    return out


@jax.jit
def pallas_concat_heads__gqa_block_cached__mha_block_cached__near_ridge_kernel(
    A_x: jax.Array,
    A_k_cache: jax.Array,
    A_v_cache: jax.Array,
    A_wq: jax.Array,
    A_wo: jax.Array,
    B_x: jax.Array,
    B_k_cache: jax.Array,
    B_v_cache: jax.Array,
    B_wq: jax.Array,
    B_wo: jax.Array,
):
    B, Sq, D = A_x.shape
    Dh = _DH
    NJ, Sk = A_k_cache.shape[1], A_k_cache.shape[2]
    rep = _HQ // NJ
    W = rep * Dh
    R = B * Sq
    NTL = R // 128
    PPJ = B // 2
    NP = NJ * PPJ
    NST = NJ * B
    L, DP, NSP, UPB = _L, _DP, _NSP, _UPB
    NQ = DP // 2
    NMIX = NP - DP - 1
    NPB = NP - 2 - NMIX
    HD = D // 2
    KC = Sk // 128
    RA = rep * Sq
    CA = D // 128 * 128
    X0 = B // 2
    assert (B, NJ, rep, NTL) == (8, 8, 2, 7) and R == NTL * 128 and Sq % 16 == 0 and HD % 16 == 0
    assert B_k_cache.shape[1] == _HQ and DP <= L < NSP - 1 and NMIX + L >= NP - 2
    qscale = Dh ** -0.5
    bf16, f32 = jnp.bfloat16, jnp.float32

    S_X = 0
    S_WQ = S_X + 3
    S_WO = S_WQ + 4
    S_A = S_WO + 1
    S_B = S_A + NSP
    S_F = S_B + NSP
    S_OUT = S_F + 5
    NSEM = S_OUT + 2 * NTL

    sched = next(s for s in (_schedule(B, NJ, NTL, DP, n) for n in range(2 * NTL, -1, -1)) if s is not None)
    table = [u for blk in sched[NQ:NQ + NMIX] for u in blk]
    a_last, tail = sched[NQ + NMIX], sched[NQ + NMIX + 1:]

    def body(xa_h, ka_h, va_h, wqa_h, woa_h, xb_h, kb_h, vb_h, wqb_h, wob_h, out_h,
             x_v, wq_v, wo_v, ka_v, va_v, kb_v, vb_v, q_v, o_v, acc_v, ost_v, s_v, p_v, tab, sem):

        def mo(v, m):
            return v if isinstance(v, int) else pl.multiple_of(v, m)

        def shr(v, n):
            return v >> n if isinstance(v, int) else lax.shift_right_logical(v, n)

        def psplit(a):
            ri = a & (NSP - 1)
            return shr(a, 2), (a & (PPJ - 1)) * 2, ri * 2, ri

        def a_copies(a):
            j, b0, sl, ri = psplit(a)
            sm = sem.at[S_A + ri]
            return (pltpu.make_async_copy(ka_h.at[pl.ds(b0, 2), j], ka_v.at[pl.ds(sl, 2)], sm),
                    pltpu.make_async_copy(va_h.at[pl.ds(b0, 2), j], va_v.at[pl.ds(sl, 2)], sm))

        def b_copies(a):
            j, b0, sl, ri = psplit(a)
            sm = sem.at[S_B + ri]
            hs = pl.ds(j * rep, rep)
            return (pltpu.make_async_copy(kb_h.at[pl.ds(b0, 2), hs], kb_v.at[pl.ds(sl, 2)], sm),
                    pltpu.make_async_copy(vb_h.at[pl.ds(b0, 2), hs], vb_v.at[pl.ds(sl, 2)], sm))

        def fine_copy(st, isv):
            j, b0, sl, _ = psplit(st // 2)
            src, dst = ((kb_h, kb_v), (vb_h, vb_v))[isv]
            si = st - (NST - 4) + (isv if st == NST - 1 else 0)
            return pltpu.make_async_copy(src.at[b0 + st % 2, pl.ds(j * rep, rep)], dst.at[sl + st % 2],
                                         sem.at[S_F + si])

        def x_copy(i):
            src, br, r0, r1 = ((xa_h, 0, 0, X0 * Sq), (xa_h, 0, X0 * Sq, R), (xb_h, 1, 0, R))[i]
            return pltpu.make_async_copy(src.at[r0:r1], x_v.at[br, r0:r1], sem.at[S_X + i])

        def wq_copy(i):
            src, br, c0, c1 = ((wqa_h, 0, 0, W), (wqa_h, 0, W, 2 * W), (wqa_h, 0, 2 * W, NJ * W),
                               (wqb_h, 1, 0, NJ * W))[i]
            return pltpu.make_async_copy(src.at[:, c0:c1], wq_v.at[br, :, c0:c1], sem.at[S_WQ + i])

        def wo_copy(br):
            return pltpu.make_async_copy((woa_h, wob_h)[br], wo_v.at[br], sem.at[S_WO])

        def cols(part):
            return {None: (0, 2 * D), 0: (0, CA), 1: (CA, 2 * D)}[part]

        def out_copy(t, part):
            c0, c1 = cols(part)
            return pltpu.make_async_copy(ost_v.at[t, :, c0:c1], out_h.at[t * 128:(t + 1) * 128, c0:c1],
                                         sem.at[S_OUT + t + (NTL if part == 0 else 0)])

        def issue(m):
            def start_a():
                for c in a_copies(m):
                    c.start()

            def start_b():
                for c in b_copies(m - DP):
                    c.start()

            if isinstance(m, int):
                if m < NP:
                    start_a()
                if 0 <= m - DP < NP - 2:
                    start_b()
            else:
                pl.when(m < NP)(start_a)
                pl.when(m - DP < NP - 2)(start_b)

        def wait_a(a):
            for c in a_copies(a):
                c.wait()

        def wait_b(a):
            for c in b_copies(a):
                c.wait()

        def qproj(br, j, b0, nb):
            x = x_v[br, b0 * Sq:(b0 + nb) * Sq, :]
            q = jnp.dot(x, wq_v[br, :, pl.ds(mo(j * W, W), W)], preferred_element_type=f32)
            q = (q * qscale).astype(bf16)
            for bb in range(nb):
                for h in range(rep):
                    q_v[br, j, b0 + bb, h] = q[bb * Sq:(bb + 1) * Sq, h * Dh:(h + 1) * Dh]

        def ounit(br, j, t, rh, nr):
            w0 = mo(rh * HD, 16)
            ot = o_v[br, pl.ds(mo(t * 128, 128), 128), :]
            lhs = wo_v[br, pl.ds(w0, nr), pl.ds(mo(j * W, W), W)]
            acc_v[t, pl.ds(mo(br * D + w0, 8), nr), :] += lax.dot_general(lhs, ot, _NT, preferred_element_type=f32)

        def table_unit(i):
            e = tab[i]
            ounit(e & 1, shr(e, 1) & 7, shr(e, 4) & 7, shr(e, 7), HD)

        def static_units(us):
            us = list(us)
            while us:
                br, j, t, rh = us.pop(0)
                if us and rh == 0 and us[0] == (br, j, t, 1):
                    us.pop(0)
                    ounit(br, j, t, 0, D)
                else:
                    ounit(br, j, t, rh, HD)

        def finalize(t, part):
            c0, c1 = cols(part)
            ost_v[t, :, c0:c1] = acc_v[t, c0:c1, :].T.astype(ost_v.dtype)

        def a_item(a, k, r0):
            j, b0, sl, _ = psplit(a)
            return (0, j, b0 + k, sl + k, None, r0)

        def b_items(a, k, r0):
            j, b0, sl, _ = psplit(a)
            return [(1, j, b0 + k, sl + k, h, r0 + h * Sq) for h in range(rep)]

        def scores(items):
            res = []
            for it in items:
                br, j, b, slot, h, r0 = it
                if br == 0:
                    q, k = q_v[0, j, b].reshape(RA, Dh), ka_v[slot]
                else:
                    q, k = q_v[1, j, b, h], kb_v[slot, h]
                s = lax.dot_general(q, k, _NT, preferred_element_type=f32)
                m = jnp.max(s, axis=-1, keepdims=True)
                s_v[r0:r0 + q.shape[0], :] = s.astype(bf16).astype(f32)
                res.append((it, q.shape[0], m.astype(bf16).astype(f32)))
            return res

        def softmax(res):
            out = []
            for it, n, m in res:
                r0 = it[5]
                p = jnp.exp(s_v[r0:r0 + n, :] - m)
                denom = jnp.sum(p, axis=-1, keepdims=True)
                p = p.astype(bf16)
                for c in range(KC):
                    p_v[c, r0:r0 + n, :] = p[:, c * 128:(c + 1) * 128]
                out.append((it, n, 1.0 / denom))
            return out

        def values(res):
            for it, n, rinv in res:
                br, j, b, slot, h, r0 = it
                rows = pl.ds(mo(b * Sq, 16), Sq)
                v = va_v[slot] if br == 0 else vb_v[slot, h]
                p = jnp.concatenate([p_v[c, r0:r0 + n, :] for c in range(KC)], axis=1)
                o = (jnp.dot(p, v, preferred_element_type=f32) * rinv).astype(bf16)
                if br == 0:
                    for hh in range(rep):
                        o_v[0, rows, hh * Dh:(hh + 1) * Dh] = o[hh * Sq:(hh + 1) * Sq]
                else:
                    o_v[1, rows, h * Dh:(h + 1) * Dh] = o

        for c in (wq_copy(0), x_copy(0), x_copy(1), wq_copy(1), wq_copy(2), x_copy(2), wq_copy(3),
                  wo_copy(0), wo_copy(1)):
            c.start()
        for m in range(L):
            issue(m)
        for i, (br, j, t, rh) in enumerate(table):
            tab[i] = br | (j << 1) | (t << 4) | (rh << 7)
        acc_v[...] = jnp.zeros(acc_v.shape, acc_v.dtype)

        nch = 2 * NJ - NQ
        n_it = (nch - 2) // _P1C
        c_first = nch - n_it * _P1C
        wq_copy(0).wait()
        x_copy(0).wait()
        qproj(0, 0, 0, X0)
        x_copy(1).wait()
        wq_copy(1).wait()
        qproj(0, 0, X0, B - X0)
        qproj(0, 1, 0, B)
        wq_copy(2).wait()
        for c in range(2, c_first):
            qproj(0, c, 0, B)

        def qproj_step(i, carry):
            c0 = c_first + i * _P1C

            @pl.when(jnp.logical_and(c0 <= NJ, c0 + _P1C > NJ))
            def _():
                x_copy(2).wait()
                wq_copy(3).wait()

            for k in range(_P1C):
                qproj(shr(c0 + k, 3), (c0 + k) & (NJ - 1), 0, B)
            return carry

        lax.fori_loop(0, n_it, qproj_step, 0)

        for br in range(2):
            wo_copy(br).wait()
        for blk in range(NQ):
            jq = NJ - NQ + blk
            wait_a(2 * blk)
            wait_a(2 * blk + 1)
            its = [a_item(2 * blk + (i >> 1), i & 1, i * RA) for i in range(4)]
            s01 = scores(its[:2])
            static_units(sched[blk])
            s23 = scores(its[2:])
            qproj(1, jq, 0, B // 2)
            values(softmax(s01))
            issue(L + 2 * blk)
            values(softmax(s23))
            issue(L + 2 * blk + 1)
            qproj(1, jq, B // 2, B // 2)

        def mixed(n, carry):
            a = n + DP
            wait_a(a)
            wait_b(n)
            s0 = scores([a_item(a, 0, 0)])
            table_unit(n * UPB)
            s0 += scores(b_items(n, 0, RA))
            for i in range(1, 3):
                table_unit(n * UPB + i)
            s1 = scores([a_item(a, 1, 2 * RA)])
            table_unit(n * UPB + 3)
            s1 += scores(b_items(n, 1, 3 * RA))
            for i in range(4, UPB):
                table_unit(n * UPB + i)
            values(softmax(s0))
            issue(a + L)
            values(softmax(s1))
            return carry

        lax.fori_loop(0, NMIX, mixed, 0)

        def pair_block(items0, items1, us):
            cut = (len(us) + 2) // 4 * 2
            s0 = scores(items0)
            static_units(us[:cut])
            s1 = scores(items1)
            static_units(us[cut:])
            values(softmax(s0))
            values(softmax(s1))

        for st in range(NST - 4, NST):
            for isv in range(2):
                fine_copy(st, isv).start()
        wait_a(NP - 1)
        pair_block([a_item(NP - 1, 0, 0)], [a_item(NP - 1, 1, RA)], a_last)
        for blk in range(NPB):
            a = NMIX + blk
            wait_b(a)
            pair_block(b_items(a, 0, 0), b_items(a, 1, RA), tail[blk])

        fine = tail[NPB:]
        done_at = {t: -1 for t in range(NTL)}
        for si, us in enumerate(fine):
            for br, j, t, _ in us:
                assert br == 1 and j == NJ - 1
                done_at[t] = si
        split = range(NTL - _NSPLIT, NTL)

        def part(t):
            return 1 if t in split else None

        def flush(si):
            if si == 0:
                for t in split:
                    finalize(t, 0)
            for t in range(NTL - 1):
                if done_at[t] + 1 == si:
                    finalize(t, part(t))
            for t in range(NTL - 1):
                assert _OUT_STAGE[t] > done_at[t]
                if _OUT_STAGE[t] == si:
                    out_copy(t, part(t)).start()
            if si == 0:
                for t in split:
                    out_copy(t, 0).start()

        for si in range(3):
            st = NST - 4 + si
            fine_copy(st, 0).wait()
            fine_copy(st, 1).wait()
            s0 = scores(b_items(st // 2, st % 2, 0))
            static_units(fine[si])
            flush(si)
            values(softmax(s0))
        st = NST - 1
        fine_copy(st, 0).wait()
        s0 = scores(b_items(st // 2, st % 2, 0))
        static_units(fine[3])
        flush(3)
        p0 = softmax(s0)
        fine_copy(st, 1).wait()
        values(p0)
        flush(4)
        static_units(fine[4])
        finalize(NTL - 1, part(NTL - 1))
        out_copy(NTL - 1, part(NTL - 1)).start()
        for t in range(NTL):
            out_copy(t, part(t)).wait()
        for t in split:
            out_copy(t, 0).wait()

    hbm = pl.BlockSpec(memory_space=pltpu.HBM)
    out = pl.pallas_call(
        body,
        in_specs=[hbm] * 10,
        out_specs=hbm,
        out_shape=jax.ShapeDtypeStruct((R, 2 * D), A_x.dtype),
        scratch_shapes=[
            pltpu.VMEM((2, R, D), bf16),
            pltpu.VMEM((2, D, NJ * W), bf16),
            pltpu.VMEM((2, D, NJ * W), bf16),
            pltpu.VMEM((2 * NSP, Sk, Dh), bf16),
            pltpu.VMEM((2 * NSP, Sk, Dh), bf16),
            pltpu.VMEM((2 * NSP, rep, Sk, Dh), bf16),
            pltpu.VMEM((2 * NSP, rep, Sk, Dh), bf16),
            pltpu.VMEM((2, NJ, B, rep, Sq, Dh), bf16),
            pltpu.VMEM((2, R, W), bf16),
            pltpu.VMEM((NTL, 2 * D, 128), f32),
            pltpu.VMEM((NTL, 128, 2 * D), A_x.dtype),
            pltpu.VMEM((4 * RA, Sk), f32),
            pltpu.VMEM((KC, 4 * RA, 128), bf16),
            pltpu.SMEM((len(table),), jnp.int32),
            pltpu.SemaphoreType.DMA((NSEM,)),
        ],
        compiler_params=pltpu.CompilerParams(
            vmem_limit_bytes=120 * 1024 * 1024,
            disable_bounds_checks=True,
            disable_semaphore_checks=True,
        ),
    )(A_x.reshape(R, D), A_k_cache, A_v_cache, A_wq, A_wo.T,
      B_x.reshape(R, D), B_k_cache, B_v_cache, B_wq, B_wo.T)
    return out.reshape(B, Sq, 2 * D)
```

```python
import jax
import jax.numpy as jnp
from jax import lax
import jax.experimental.pallas as pl
import jax.experimental.pallas.tpu as pltpu

_NT = (((1,), (1,)), ((), ()))

_HQ, _DH = 16, 256
_L = 10
_DP = 4
_P1C = 4
_NSP = 16
_UNIT_PATTERN = (1, 1, 1, 1, 1, 2)
_UPB = sum(_UNIT_PATTERN)
_OUT_STAGE = (2, 2, 2, 2, 3, 4)
_NSPLIT = 2


def _schedule(B, NJ, NTL, DP, last_pa):
    NP, NST, NQ = NJ * B // 2, NJ * B, DP // 2
    NMIX = NP - DP - 1
    blocks = [(-1 if k < NQ - 1 else last_pa, 4 * k, 0, 4 * k + 4, 0) for k in range(NQ)]
    blocks += [(_UPB, 2 * (m + DP), 2 * m, 2 * (m + DP + 1), 2 * (m + 1)) for m in range(NMIX)]
    blocks += [(-1, NST - 2, 2 * NMIX, NST, 2 * NMIX)]
    blocks += [(-1, NST, 2 * m, NST, 2 * m + 2) for m in range(NMIX, NP - 2)]
    blocks += [(-1, NST, s, NST, min(s + 1, NST - 1)) for s in range(NST - 4, NST)]
    blocks += [(-1, NST, NST, NST, NST)]
    queue, pushed, out = [], [0, 0], []
    for n, da, db, ea, eb in blocks:
        for br, done in ((0, da), (1, db)):
            ready = (done // B) * NTL + max(0, done % B - 1)
            while pushed[br] < ready:
                j, t = divmod(pushed[br], NTL)
                pushed[br] += 1
                queue += [(br, j, t, 0), (br, j, t, 1)]
        queue.sort(key=lambda u: (u[1] * B + u[2] - (2 * DP if u[0] == 0 else 0), u[0], u[3]))
        if n < 0:
            n = len(queue)
        if len(queue) < n:
            return None
        out.append(queue[:n])
        queue = queue[n:]
        if any((ea, eb)[br] > (j + 1) * B + t for br, j, t, _ in queue):
            return None
    assert not queue and pushed == [NJ * NTL] * 2
    return out


@jax.jit
def pallas_concat_heads__gqa_block_cached__mha_block_cached__near_ridge_kernel(
    A_x: jax.Array,
    A_k_cache: jax.Array,
    A_v_cache: jax.Array,
    A_wq: jax.Array,
    A_wo: jax.Array,
    B_x: jax.Array,
    B_k_cache: jax.Array,
    B_v_cache: jax.Array,
    B_wq: jax.Array,
    B_wo: jax.Array,
):
    B, Sq, D = A_x.shape
    Dh = _DH
    NJ, Sk = A_k_cache.shape[1], A_k_cache.shape[2]
    rep = _HQ // NJ
    W = rep * Dh
    R = B * Sq
    NTL = R // 128
    PPJ = B // 2
    NP = NJ * PPJ
    NST = NJ * B
    L, DP, NSP, UPB = _L, _DP, _NSP, _UPB
    NQ = DP // 2
    NMIX = NP - DP - 1
    NPB = NP - 2 - NMIX
    HD = D // 2
    KC = Sk // 128
    RA = rep * Sq
    CA = D // 128 * 128
    X0 = B // 2
    assert (B, NJ, rep, NTL) == (8, 8, 2, 7) and R == NTL * 128 and Sq % 16 == 0 and HD % 16 == 0
    assert B_k_cache.shape[1] == _HQ and DP <= L < NSP - 1 and NMIX + L >= NP - 2
    qscale = Dh ** -0.5
    bf16, f32 = jnp.bfloat16, jnp.float32

    S_X = 0
    S_WQ = S_X + 3
    S_WO = S_WQ + 4
    S_A = S_WO + 1
    S_B = S_A + NSP
    S_F = S_B + NSP
    S_OUT = S_F + 5
    NSEM = S_OUT + 2 * NTL

    sched = next(s for s in (_schedule(B, NJ, NTL, DP, n) for n in range(2 * NTL, -1, -1)) if s is not None)
    table = [u for blk in sched[NQ:NQ + NMIX] for u in blk]
    a_last, tail = sched[NQ + NMIX], sched[NQ + NMIX + 1:]

    def body(xa_h, ka_h, va_h, wqa_h, woa_h, xb_h, kb_h, vb_h, wqb_h, wob_h, out_h,
             x_v, wq_v, wo_v, ka_v, va_v, kb_v, vb_v, q_v, o_v, acc_v, ost_v, s_v, p_v, tab, sem):

        def mo(v, m):
            return v if isinstance(v, int) else pl.multiple_of(v, m)

        def shr(v, n):
            return v >> n if isinstance(v, int) else lax.shift_right_logical(v, n)

        def psplit(a):
            ri = a & (NSP - 1)
            return shr(a, 2), (a & (PPJ - 1)) * 2, ri * 2, ri

        def a_copies(a):
            j, b0, sl, ri = psplit(a)
            sm = sem.at[S_A + ri]
            return (pltpu.make_async_copy(ka_h.at[pl.ds(b0, 2), j], ka_v.at[pl.ds(sl, 2)], sm),
                    pltpu.make_async_copy(va_h.at[pl.ds(b0, 2), j], va_v.at[pl.ds(sl, 2)], sm))

        def b_copies(a):
            j, b0, sl, ri = psplit(a)
            sm = sem.at[S_B + ri]
            hs = pl.ds(j * rep, rep)
            return (pltpu.make_async_copy(kb_h.at[pl.ds(b0, 2), hs], kb_v.at[pl.ds(sl, 2)], sm),
                    pltpu.make_async_copy(vb_h.at[pl.ds(b0, 2), hs], vb_v.at[pl.ds(sl, 2)], sm))

        def fine_copy(st, isv):
            j, b0, sl, _ = psplit(st // 2)
            src, dst = ((kb_h, kb_v), (vb_h, vb_v))[isv]
            si = st - (NST - 4) + (isv if st == NST - 1 else 0)
            return pltpu.make_async_copy(src.at[b0 + st % 2, pl.ds(j * rep, rep)], dst.at[sl + st % 2],
                                         sem.at[S_F + si])

        def x_copy(i):
            src, br, r0, r1 = ((xa_h, 0, 0, X0 * Sq), (xa_h, 0, X0 * Sq, R), (xb_h, 1, 0, R))[i]
            return pltpu.make_async_copy(src.at[r0:r1], x_v.at[br, r0:r1], sem.at[S_X + i])

        def wq_copy(i):
            src, br, c0, c1 = ((wqa_h, 0, 0, W), (wqa_h, 0, W, 2 * W), (wqa_h, 0, 2 * W, NJ * W),
                               (wqb_h, 1, 0, NJ * W))[i]
            return pltpu.make_async_copy(src.at[:, c0:c1], wq_v.at[br, :, c0:c1], sem.at[S_WQ + i])

        def wo_copy(br):
            return pltpu.make_async_copy((woa_h, wob_h)[br], wo_v.at[br], sem.at[S_WO])

        def cols(part):
            return {None: (0, 2 * D), 0: (0, CA), 1: (CA, 2 * D)}[part]

        def out_copy(t, part):
            c0, c1 = cols(part)
            return pltpu.make_async_copy(ost_v.at[t, :, c0:c1], out_h.at[t * 128:(t + 1) * 128, c0:c1],
                                         sem.at[S_OUT + t + (NTL if part == 0 else 0)])

        def issue(m):
            def start_a():
                for c in a_copies(m):
                    c.start()

            def start_b():
                for c in b_copies(m - DP):
                    c.start()

            if isinstance(m, int):
                if m < NP:
                    start_a()
                if 0 <= m - DP < NP - 2:
                    start_b()
            else:
                pl.when(m < NP)(start_a)
                pl.when(m - DP < NP - 2)(start_b)

        def wait_a(a):
            for c in a_copies(a):
                c.wait()

        def wait_b(a):
            for c in b_copies(a):
                c.wait()

        def qproj(br, j, b0, nb):
            x = x_v[br, b0 * Sq:(b0 + nb) * Sq, :]
            q = jnp.dot(x, wq_v[br, :, pl.ds(mo(j * W, W), W)], preferred_element_type=f32)
            q = (q * qscale).astype(bf16)
            for bb in range(nb):
                for h in range(rep):
                    q_v[br, j, b0 + bb, h] = q[bb * Sq:(bb + 1) * Sq, h * Dh:(h + 1) * Dh]

        def ounit(br, j, t, rh, nr):
            w0 = mo(rh * HD, 16)
            ot = o_v[br, pl.ds(mo(t * 128, 128), 128), :]
            lhs = wo_v[br, pl.ds(w0, nr), pl.ds(mo(j * W, W), W)]
            acc_v[t, pl.ds(mo(br * D + w0, 8), nr), :] += lax.dot_general(lhs, ot, _NT, preferred_element_type=f32)

        def table_unit(i):
            e = tab[i]
            ounit(e & 1, shr(e, 1) & 7, shr(e, 4) & 7, shr(e, 7), HD)

        def static_units(us):
            us = list(us)
            while us:
                br, j, t, rh = us.pop(0)
                if us and rh == 0 and us[0] == (br, j, t, 1):
                    us.pop(0)
                    ounit(br, j, t, 0, D)
                else:
                    ounit(br, j, t, rh, HD)

        def finalize(t, part):
            c0, c1 = cols(part)
            ost_v[t, :, c0:c1] = acc_v[t, c0:c1, :].T.astype(ost_v.dtype)

        def a_item(a, k, r0):
            j, b0, sl, _ = psplit(a)
            return (0, j, b0 + k, sl + k, None, r0)

        def b_items(a, k, r0):
            j, b0, sl, _ = psplit(a)
            return [(1, j, b0 + k, sl + k, h, r0 + h * Sq) for h in range(rep)]

        def scores(items):
            res = []
            for it in items:
                br, j, b, slot, h, r0 = it
                if br == 0:
                    q, k = q_v[0, j, b].reshape(RA, Dh), ka_v[slot]
                else:
                    q, k = q_v[1, j, b, h], kb_v[slot, h]
                s = lax.dot_general(q, k, _NT, preferred_element_type=f32)
                m = jnp.max(s, axis=-1, keepdims=True)
                s_v[r0:r0 + q.shape[0], :] = s.astype(bf16).astype(f32)
                res.append((it, q.shape[0], m.astype(bf16).astype(f32)))
            return res

        def softmax(res):
            out = []
            for it, n, m in res:
                r0 = it[5]
                p = jnp.exp(s_v[r0:r0 + n, :] - m)
                denom = jnp.sum(p, axis=-1, keepdims=True)
                p = p.astype(bf16)
                for c in range(KC):
                    p_v[c, r0:r0 + n, :] = p[:, c * 128:(c + 1) * 128]
                out.append((it, n, 1.0 / denom))
            return out

        def values(res):
            for it, n, rinv in res:
                br, j, b, slot, h, r0 = it
                rows = pl.ds(mo(b * Sq, 16), Sq)
                v = va_v[slot] if br == 0 else vb_v[slot, h]
                p = jnp.concatenate([p_v[c, r0:r0 + n, :] for c in range(KC)], axis=1)
                o = (jnp.dot(p, v, preferred_element_type=f32) * rinv).astype(bf16)
                if br == 0:
                    for hh in range(rep):
                        o_v[0, rows, hh * Dh:(hh + 1) * Dh] = o[hh * Sq:(hh + 1) * Sq]
                else:
                    o_v[1, rows, h * Dh:(h + 1) * Dh] = o

        for c in (wq_copy(0), x_copy(0), x_copy(1), wq_copy(1), wq_copy(2), x_copy(2), wq_copy(3),
                  wo_copy(0), wo_copy(1)):
            c.start()
        for m in range(L):
            issue(m)
        for i, (br, j, t, rh) in enumerate(table):
            tab[i] = br | (j << 1) | (t << 4) | (rh << 7)
        acc_v[...] = jnp.zeros(acc_v.shape, acc_v.dtype)

        nch = 2 * NJ - NQ
        n_it = (nch - 2) // _P1C
        c_first = nch - n_it * _P1C
        wq_copy(0).wait()
        x_copy(0).wait()
        qproj(0, 0, 0, X0)
        x_copy(1).wait()
        wq_copy(1).wait()
        qproj(0, 0, X0, B - X0)
        qproj(0, 1, 0, B)
        wq_copy(2).wait()
        for c in range(2, c_first):
            qproj(0, c, 0, B)

        def qproj_step(i, carry):
            c0 = c_first + i * _P1C

            @pl.when(jnp.logical_and(c0 <= NJ, c0 + _P1C > NJ))
            def _():
                x_copy(2).wait()
                wq_copy(3).wait()

            for k in range(_P1C):
                qproj(shr(c0 + k, 3), (c0 + k) & (NJ - 1), 0, B)
            return carry

        lax.fori_loop(0, n_it, qproj_step, 0)

        for br in range(2):
            wo_copy(br).wait()
        for blk in range(NQ):
            jq = NJ - NQ + blk
            wait_a(2 * blk)
            wait_a(2 * blk + 1)
            its = [a_item(2 * blk + (i >> 1), i & 1, i * RA) for i in range(4)]
            s01 = scores(its[:2])
            static_units(sched[blk])
            s23 = scores(its[2:])
            qproj(1, jq, 0, B // 2)
            values(softmax(s01))
            issue(L + 2 * blk)
            values(softmax(s23))
            issue(L + 2 * blk + 1)
            qproj(1, jq, B // 2, B // 2)

        def mixed(n, carry):
            a = n + DP
            wait_a(a)
            wait_b(n)
            items = [a_item(a, 0, 0)] + b_items(n, 0, RA) + [a_item(a, 1, 2 * RA)] + b_items(n, 1, 3 * RA)
            sc, u = [], 0
            for it, nu in zip(items, _UNIT_PATTERN):
                sc.append(scores([it]))
                for _ in range(nu):
                    table_unit(n * UPB + u)
                    u += 1
            for i, s_i in enumerate(sc):
                if i == len(sc) // 2:
                    issue(a + L)
                values(softmax(s_i))
            return carry

        lax.fori_loop(0, NMIX, mixed, 0)

        def pair_block(items0, items1, us):
            cut = (len(us) + 2) // 4 * 2
            s0 = scores(items0)
            static_units(us[:cut])
            s1 = scores(items1)
            static_units(us[cut:])
            values(softmax(s0))
            values(softmax(s1))

        for st in range(NST - 4, NST):
            for isv in range(2):
                fine_copy(st, isv).start()
        wait_a(NP - 1)
        pair_block([a_item(NP - 1, 0, 0)], [a_item(NP - 1, 1, RA)], a_last)
        for blk in range(NPB):
            a = NMIX + blk
            wait_b(a)
            pair_block(b_items(a, 0, 0), b_items(a, 1, RA), tail[blk])

        fine = tail[NPB:]
        done_at = {t: -1 for t in range(NTL)}
        for si, us in enumerate(fine):
            for br, j, t, _ in us:
                assert br == 1 and j == NJ - 1
                done_at[t] = si
        split = range(NTL - _NSPLIT, NTL)

        def part(t):
            return 1 if t in split else None

        def flush(si):
            if si == 0:
                for t in split:
                    finalize(t, 0)
            for t in range(NTL - 1):
                if done_at[t] + 1 == si:
                    finalize(t, part(t))
            for t in range(NTL - 1):
                assert _OUT_STAGE[t] > done_at[t]
                if _OUT_STAGE[t] == si:
                    out_copy(t, part(t)).start()
            if si == 0:
                for t in split:
                    out_copy(t, 0).start()

        for si in range(3):
            st = NST - 4 + si
            fine_copy(st, 0).wait()
            fine_copy(st, 1).wait()
            s0 = scores(b_items(st // 2, st % 2, 0))
            static_units(fine[si])
            flush(si)
            values(softmax(s0))
        st = NST - 1
        fine_copy(st, 0).wait()
        s0 = scores(b_items(st // 2, st % 2, 0))
        static_units(fine[3])
        flush(3)
        p0 = softmax(s0)
        fine_copy(st, 1).wait()
        values(p0)
        flush(4)
        static_units(fine[4])
        finalize(NTL - 1, part(NTL - 1))
        out_copy(NTL - 1, part(NTL - 1)).start()
        for t in range(NTL):
            out_copy(t, part(t)).wait()
        for t in split:
            out_copy(t, 0).wait()

    hbm = pl.BlockSpec(memory_space=pltpu.HBM)
    out = pl.pallas_call(
        body,
        in_specs=[hbm] * 10,
        out_specs=hbm,
        out_shape=jax.ShapeDtypeStruct((R, 2 * D), A_x.dtype),
        scratch_shapes=[
            pltpu.VMEM((2, R, D), bf16),
            pltpu.VMEM((2, D, NJ * W), bf16),
            pltpu.VMEM((2, D, NJ * W), bf16),
            pltpu.VMEM((2 * NSP, Sk, Dh), bf16),
            pltpu.VMEM((2 * NSP, Sk, Dh), bf16),
            pltpu.VMEM((2 * NSP, rep, Sk, Dh), bf16),
            pltpu.VMEM((2 * NSP, rep, Sk, Dh), bf16),
            pltpu.VMEM((2, NJ, B, rep, Sq, Dh), bf16),
            pltpu.VMEM((2, R, W), bf16),
            pltpu.VMEM((NTL, 2 * D, 128), f32),
            pltpu.VMEM((NTL, 128, 2 * D), A_x.dtype),
            pltpu.VMEM((4 * RA, Sk), f32),
            pltpu.VMEM((KC, 4 * RA, 128), bf16),
            pltpu.SMEM((len(table),), jnp.int32),
            pltpu.SemaphoreType.DMA((NSEM,)),
        ],
        compiler_params=pltpu.CompilerParams(
            vmem_limit_bytes=120 * 1024 * 1024,
            disable_bounds_checks=True,
            disable_semaphore_checks=True,
        ),
    )(A_x.reshape(R, D), A_k_cache, A_v_cache, A_wq, A_wo.T,
      B_x.reshape(R, D), B_k_cache, B_v_cache, B_wq, B_wo.T)
    return out.reshape(B, Sq, 2 * D)
```
